```python
import jax
import jax.numpy as jnp

def _softmax(x, axis=-1):
    return jax.nn.softmax(x, axis=axis)
def _gelu(x):
    return jax.nn.gelu(x, approximate=True)
def _silu(x):
    return jax.nn.silu(x)
def _sigmoid(x):
    return jax.nn.sigmoid(x)
def _layernorm(x, axis=-1, eps=1e-5):
    m = jnp.mean(x, axis=axis, keepdims=True)
    v = jnp.var(x, axis=axis, keepdims=True)
    return (x - m) / jnp.sqrt(v + eps)
def _scatter_add(tgt, idx, src, axis=0):
    return tgt.at[idx].add(src)
def _segment_sum(src, seg, n):
    return jax.ops.segment_sum(src, seg, n)
class _Rng:
    def __init__(self, key):
        self._k = key
    def _next(self):
        self._k, sub = jax.random.split(self._k)
        return sub
    def normal(self, shape):
        return jax.random.normal(self._next(), shape, dtype=jnp.bfloat16)
    def randint(self, lo, hi, shape):
        return jax.random.randint(self._next(), shape, lo, hi, dtype=jnp.int32)
    def uniform(self, shape, lo=0.0, hi=1.0):
        return jax.random.uniform(self._next(), shape, jnp.bfloat16, lo, hi)
    def permutation(self, n):
        return jax.random.permutation(self._next(), n)


kernel_name = 'interleave_layers__sliding_block_cached__moe_arch_mod__decode'

def setup_inputs():
    _rng = _Rng(jax.random.key(int.from_bytes(__import__("os").urandom(4), "little")))
    _w = (lambda a: (lambda t: t.astype(jnp.bfloat16) if jnp.issubdtype(t.dtype, jnp.floating) else t)(jnp.asarray(a)))
    def _A_setup():
        B, Sq, D = 4, 1, 640
        Hq, Hkv, Sk, Dh = 32, 32, 4096, 192
        assert Hq % Hkv == 0, (Hq, Hkv)
        return {
            "x": _w((lambda *s: _rng.normal(s) * 0.05)(B, Sq, D)),
            "k_cache": _w((lambda *s: _rng.normal(s) * 0.05)(B, Hkv, Sk, Dh)),
            "v_cache": _w((lambda *s: _rng.normal(s) * 0.05)(B, Hkv, Sk, Dh)),
            "wq": _w((lambda *s: _rng.normal(s) * 0.05)(D, Hq * Dh) * (D ** -0.5)),
            "wo": _w((lambda *s: _rng.normal(s) * 0.05)(Hq * Dh, D) * ((Hq * Dh) ** -0.5)),
        }
    _A_in = _A_setup()

    def _B_setup():
        B, S, D, F, C = 4, 1, 640, 1536, 1
        return {
            "x": _w((lambda *s: _rng.normal(s) * 0.05)(B, S, D)),
            "w_r": _w((lambda *s: _rng.normal(s) * 0.05)(D)),
            "w_gate": _w((lambda *s: _rng.normal(s) * 0.05)(D, F)),
            "w_up": _w((lambda *s: _rng.normal(s) * 0.05)(D, F)),
            "w_down": _w((lambda *s: _rng.normal(s) * 0.05)(F, D)),
        }
    _B_in = _B_setup()

    return {
        "A_x": _A_in["x"],
        "A_k_cache": _A_in["k_cache"],
        "A_v_cache": _A_in["v_cache"],
        "A_wq": _A_in["wq"],
        "A_wo": _A_in["wo"],
        "B_x": _B_in["x"],
        "B_w_r": _B_in["w_r"],
        "B_w_gate": _B_in["w_gate"],
        "B_w_up": _B_in["w_up"],
        "B_w_down": _B_in["w_down"],
    }

def reference(A_x, A_k_cache, A_v_cache, A_wq, A_wo, B_x, B_w_r, B_w_gate, B_w_up, B_w_down):
    def _A_ref(x, k_cache, v_cache, wq, wo):
        B, Sq, D = x.shape
        Hq, Dh = 32, 192
        Hkv, Sk = k_cache.shape[1], k_cache.shape[2]
        W = min(4096, max(256, Sk // 4))
        rep = Hq // Hkv
        q = (lambda x, *d: x.transpose(*d))((x @ wq).reshape(B, Sq, Hq, Dh), 0, 2, 1, 3)
        k = jnp.repeat(k_cache[:, :, Sk - W:, :], rep, axis=1)
        v = jnp.repeat(v_cache[:, :, Sk - W:, :], rep, axis=1)
        scores = jnp.einsum("bhqd,bhkd->bhqk", q, k) * (Dh ** -0.5)
        p = _softmax(scores, axis=-1)
        o = jnp.einsum("bhqk,bhkd->bhqd", p, v)
        return (lambda x, *d: x.transpose(*d))(o, 0, 2, 1, 3).reshape(B, Sq, Hq * Dh) @ wo

    def _B_ref(x, w_r, w_gate, w_up, w_down):
        B, S, D = x.shape
        C = 1
        r = x @ w_r
        idx = jnp.argsort(-r, axis=-1)[:, :C]
        idx_e = jnp.repeat(idx.reshape(B, C, 1), D, axis=2)
        x_sel = jnp.take_along_axis(x, idx_e, axis=1)
        g = _silu(x_sel @ w_gate)
        u = x_sel @ w_up
        y = (g * u) @ w_down
        r_sel = _sigmoid(jnp.take_along_axis(r, idx, axis=1))
        y = y * r_sel.reshape(B, C, 1)
        b_off = (jnp.arange(B) * S).reshape(B, 1)
        flat_idx = (idx + b_off).reshape(B * C)
        zero = (x * 0.0).reshape(B * S, D)
        upd = _scatter_add(zero, flat_idx, y.reshape(B * C, D), axis=0)
        return x + upd.reshape(B, S, D)

    x = A_x
    x = x + _A_ref(_layernorm(x, axis=-1), A_k_cache, A_v_cache, A_wq, A_wo)
    x = x + _B_ref(_layernorm(x, axis=-1), B_w_r, B_w_gate, B_w_up, B_w_down)
    x = x + _A_ref(_layernorm(x, axis=-1), A_k_cache, A_v_cache, A_wq, A_wo)
    x = x + _B_ref(_layernorm(x, axis=-1), B_w_r, B_w_gate, B_w_up, B_w_down)
    return x
```

```python
import functools
import jax
import jax.numpy as jnp
from jax import lax
import jax.experimental.pallas as pl
import jax.experimental.pallas.tpu as pltpu

B, D, H, DH, SK, W, F = 4, 640, 32, 192, 4096, 1024, 1536
NC = W // 128
SCALE = DH ** -0.5
LOG2E = 1.4426950408889634
EPS = 1e-5
BF = jnp.bfloat16
F32 = jnp.float32


def _ln(x):
    m = jnp.mean(x, axis=-1, keepdims=True)
    xc = x - m
    v = jnp.mean(xc * xc, axis=-1, keepdims=True)
    return xc / jnp.sqrt(v + EPS)


def _bf(u):
    return pltpu.bitcast(u, BF)


def default_chunks(b):
    if b < B - 1:
        return [(0, 32)], [(0, 32)]
    return [(0, 32)], [(0, 24), (24, 4), (28, 2), (30, 1), (31, 1)]


def make_kernel(late_issue=4, reduce_mode='mxu', scopes=False, unroll=1, chunks=default_chunks, pv_rows=16):
    KCH = [chunks(b)[0] for b in range(B)]
    VCH = [chunks(b)[1] for b in range(B)]
    ksizes = sorted({s for b in range(B) for (_, s) in KCH[b]})
    vsizes = sorted({s for b in range(B) for (_, s) in VCH[b]})

    def scope(name):
        import contextlib
        return jax.named_scope(name) if scopes else contextlib.nullcontext()

    def _kernel(x_hbm, k_hbm, v_hbm, wq_hbm, wo_hbm, wr_hbm, wg_hbm, wu_hbm, wd_hbm,
                out_ref,
                xb, kbuf, vbuf, wq, wo, wr, wg, wu, wd, xs, qbuf, sbuf, mbuf, pbuf, lbuf, abuf, obuf, sem_w, sem_k, sem_v):
        small = [pltpu.make_async_copy(x_hbm, xb, sem_w.at[0]), pltpu.make_async_copy(wr_hbm, wr, sem_w.at[1])]
        nat = [pltpu.make_async_copy(wq_hbm, wq, sem_w.at[2]), pltpu.make_async_copy(wg_hbm, wg, sem_w.at[4]),
               pltpu.make_async_copy(wu_hbm, wu, sem_w.at[5]), pltpu.make_async_copy(wd_hbm, wd, sem_w.at[6])]

        def wotile(n):
            return pltpu.make_async_copy(wo_hbm.at[:, pl.ds(pl.multiple_of(n * 128, 128), 128)], wo.at[n], sem_w.at[3])

        def kvtile(hbm, buf, sem, b, h0, n, c):
            return pltpu.make_async_copy(hbm.at[b, pl.ds(h0, n), :, pl.ds(pl.multiple_of(SK - W + c * 128, 128), 128)],
                                         buf.at[b, pl.ds(h0, n), c], sem.at[b, h0])

        def kvall(buf, sem, b, h0, n):
            return pltpu.make_async_copy(buf.at[b, pl.ds(h0, n)], buf.at[b, pl.ds(h0, n)], sem.at[b, h0])

        def ordered(fn):
            lax.fori_loop(0, pl.num_programs(0), lambda i, c: (fn(), c)[1], 0)

        def issue_chunk(which, b, h0, n):
            def issue_kv(c, carry):
                if which == 'k':
                    kvtile(k_hbm, kbuf, sem_k, b, h0, n, c).start()
                else:
                    kvtile(v_hbm, vbuf, sem_v, b, h0, n, c).start()
                return carry
            lax.fori_loop(0, NC, issue_kv, 0)

        for c in small + nat:
            ordered(c.start)
        lax.fori_loop(0, D // 128, lambda n, c: (wotile(n).start(), c)[1], 0)
        for b in range(B):
            for (h0, n) in KCH[b]:
                issue_chunk('k', b, h0, n)
            if b < B - 1:
                for (h0, n) in VCH[b]:
                    issue_chunk('v', b, h0, n)

        small[0].wait()
        small[1].wait()
        xs[...] = jnp.zeros((8, D), F32)
        xs[0:4, :] = xb[...].astype(F32)
        wr32 = jnp.broadcast_to(wr[...].astype(F32).reshape(1, D), (8, D))
        for c in nat:
            c.wait()
        pltpu.make_async_copy(wo, wo, sem_w.at[3]).wait()

        k32 = kbuf.bitcast(jnp.uint32)
        wo32 = wo.bitcast(jnp.uint32)

        def mm(lhs_tiles, w, n):
            out = None
            r = 0
            for a in lhs_tiles:
                kt = a.shape[1]
                d = jnp.dot(a, w[r:r + kt, n * 128:(n + 1) * 128], preferred_element_type=F32)
                out = d if out is None else out + d
                r += kt
            return out

        def split128(a):
            return [a[:, i:min(i + 128, a.shape[1])] for i in range(0, a.shape[1], 128)]

        def wait_chunk(table, buf, sem, b, h, sizes):
            for s in sizes:
                cond = None
                for bb in range(B):
                    for (h0, n) in table[bb]:
                        if n != s:
                            continue
                        if isinstance(h, int):
                            if h != h0:
                                continue
                            c = b == bb
                        else:
                            c = jnp.logical_and(b == bb, h == h0)
                        cond = c if cond is None else jnp.logical_or(cond, c)
                if cond is None:
                    continue
                hh = h if isinstance(h, int) else jnp.minimum(h, H - s)
                @pl.when(cond)
                def _():
                    kvall(buf, sem, b, hh, s).wait()

        def layer_(it, carry):
            b = it // 2
            first = (it % 2) == 0

            @pl.when(it == late_issue)
            def _():
                for (h0, n) in VCH[B - 1]:
                    issue_chunk('v', B - 1, h0, n)
            x = jnp.broadcast_to(xs[pl.ds(b, 1), :], (8, D))
            xn = _ln(x).astype(BF)
            xt = split128(xn)
            with scope('qproj'):
                for j in range(H // 2):
                    qq = jnp.concatenate([mm(xt, wq, 3 * j + t) for t in range(3)], axis=1)
                    qq = qq * (SCALE * LOG2E)
                    qbuf[2 * j, :, 0:DH] = qq[:, 0:DH].astype(BF)
                    qbuf[2 * j + 1, :, 0:DH] = qq[:, DH:2 * DH].astype(BF)

            def st_a1(h):
                q = qbuf[h, :, 0:DH]
                qa, qb = q[:, 0:128], q[:, 128:DH]
                ss = []
                for c in range(NC):
                    s = jnp.dot(qa, _bf(k32[b, h, c, 0:64, :]), preferred_element_type=F32) + \
                        jnp.dot(qb, _bf(k32[b, h, c, 64:96, :]), preferred_element_type=F32)
                    ss.append(s)
                    sbuf[h % 2, :, c * 128:(c + 1) * 128] = s
                m = ss[0]
                for s in ss[1:]:
                    m = jnp.maximum(m, s)
                mbuf[h % 2] = m

            def st_a2(h):
                m = jnp.max(mbuf[h % 2], axis=-1, keepdims=True)
                p = jnp.exp2(sbuf[h % 2] - m)
                l = jnp.sum(p, axis=-1, keepdims=True)
                pbuf[h % 2] = p
                lbuf[h % 4] = jnp.broadcast_to(1.0 / l, (8, 128))

            def st_b1(h):
                p = pbuf[h % 2]
                for r0 in range(0, DH, pv_rows):
                    a = None
                    for c in range(NC):
                        vv = vbuf[b, h, c, r0:r0 + pv_rows, :].astype(F32)
                        vv = vv.reshape(pv_rows // 8, 8, 128) * p[None, :, c * 128:(c + 1) * 128]
                        a = vv if a is None else a + vv
                    abuf[h % 2, r0:r0 + pv_rows, :] = a.reshape(pv_rows, 128).astype(abuf.dtype)

            def st_b2(h):
                A = abuf[h % 2]
                if reduce_mode == 'xlu':
                    o8 = jnp.sum(A.T.reshape(16, 8, DH), axis=0)
                else:
                    ones = jnp.full((8, 128), 0.125, BF)
                    o8 = lax.dot_general(ones, A, (((1,), (1,)), ((), ())), preferred_element_type=F32)
                il = lbuf[h % 4]
                o8 = jnp.concatenate([o8[:, 0:128] * il, o8[:, 128:DH] * il[:, 0:64]], axis=1)
                obuf[h % 2, :, 0:DH] = o8.astype(BF)

            def st_c(h, acc):
                o = obuf[h % 2, :, 0:DH]
                oa, ob = o[:, 0:128], o[:, 128:DH]
                r0 = pl.multiple_of(h * (DH // 2), 32)
                outs = []
                for n in range(D // 128):
                    y = jnp.dot(oa, _bf(wo32[n, pl.ds(r0, 64), :]), preferred_element_type=F32) + \
                        jnp.dot(ob, _bf(wo32[n, pl.ds(r0 + 64, 32), :]), preferred_element_type=F32)
                    outs.append(y)
                return acc + jnp.concatenate(outs, axis=1)

            def waits(hk, hv):
                @pl.when(first)
                def _():
                    if hk is not None:
                        wait_chunk(KCH, kbuf, sem_k, b, hk, ksizes)
                    if hv is not None:
                        wait_chunk(VCH, vbuf, sem_v, b, hv, vsizes)

            def step(i, acc, lo=0, hi=H):
                static = isinstance(i, int)
                ok = (lambda h: 0 <= h < H) if static else (lambda h: True)
                waits(i if ok(i) else None, i - 2 if ok(i - 2) else None)
                if ok(i - 4): acc = st_c(i - 4, acc)
                if ok(i - 3): st_b2(i - 3)
                if ok(i - 2): st_b1(i - 2)
                if ok(i - 1): st_a2(i - 1)
                if ok(i): st_a1(i)
                return acc

            acc = jnp.zeros((8, D), F32)
            with scope('attn'):
                for i in range(4):
                    acc = step(i, acc)
                acc = lax.fori_loop(4, H, step, acc, unroll=unroll)
                for i in range(H, H + 4):
                    acc = step(i, acc)
            with scope('ffn'):
                x = x + jnp.sum(acc, axis=0, keepdims=True)
                xnb = _ln(x).astype(BF)
                xn32 = xnb.astype(F32)
                r = jnp.sum(xn32 * wr32, axis=-1, keepdims=True)
                xt = split128(xnb)
                hs = []
                for n in range(F // 128):
                    gt = mm(xt, wg, n)
                    up = mm(xt, wu, n)
                    hs.append((gt * jax.nn.sigmoid(gt) * up).astype(BF))
                y = jnp.concatenate([mm(hs, wd, n) for n in range(D // 128)], axis=1)
                y = y * jax.nn.sigmoid(r)
                x = x + (xn32 + (xn32 * 0.0 + y))
                xs[pl.ds(b, 1), :] = x[0:1, :]
            return carry

        def layer(it, carry):
            with scope('layer'):
                return layer_(it, carry)

        lax.fori_loop(0, 2 * B, layer, 0)
        out_ref[...] = xs[0:4, :].astype(BF)

    @jax.jit
    def kernel_fn(A_x, A_k_cache, A_v_cache, A_wq, A_wo, B_x, B_w_r, B_w_gate, B_w_up, B_w_down):
        kt = jnp.swapaxes(A_k_cache, 2, 3)
        vt = jnp.swapaxes(A_v_cache, 2, 3)
        x2 = A_x.reshape(B, D)
        anyspec = pl.BlockSpec(memory_space=pl.ANY)
        out = pl.pallas_call(
            _kernel,
            out_shape=jax.ShapeDtypeStruct((B, D), BF), grid=(1,),
            in_specs=[anyspec] * 9,
            out_specs=pl.BlockSpec(memory_space=pltpu.VMEM),
            scratch_shapes=[
                pltpu.VMEM((B, D), BF),
                pltpu.VMEM((B, H, NC, DH, 128), BF),
                pltpu.VMEM((B, H, NC, DH, 128), BF),
                pltpu.VMEM((D, H * DH), BF),
                pltpu.VMEM((D // 128, H * DH, 128), BF),
                pltpu.VMEM((D,), BF),
                pltpu.VMEM((D, F), BF),
                pltpu.VMEM((D, F), BF),
                pltpu.VMEM((F, D), BF),
                pltpu.VMEM((8, D), F32),
                pltpu.VMEM((H, 8, 256), BF),
                pltpu.VMEM((2, 8, W), F32),
                pltpu.VMEM((2, 8, 128), F32),
                pltpu.VMEM((2, 8, W), F32),
                pltpu.VMEM((4, 8, 128), F32),
                pltpu.VMEM((2, DH, 128), BF if reduce_mode == 'mxu' else F32),
                pltpu.VMEM((2, 8, 256), BF),
                pltpu.SemaphoreType.DMA((7,)),
                pltpu.SemaphoreType.DMA((B, H)),
                pltpu.SemaphoreType.DMA((B, H)),
            ],
            compiler_params=pltpu.CompilerParams(vmem_limit_bytes=126 * 1024 * 1024),
        )(x2, kt, vt, A_wq, A_wo, B_w_r, B_w_gate, B_w_up, B_w_down)
        return out.reshape(B, 1, D)
    return kernel_fn


_impl = make_kernel()


@jax.jit
def pallas_interleave_layers__sliding_block_cached__moe_arch_mod__decode_kernel(
    A_x, A_k_cache, A_v_cache, A_wq, A_wo, B_x, B_w_r, B_w_gate, B_w_up, B_w_down
):
    return _impl(A_x, A_k_cache, A_v_cache, A_wq, A_wo, B_x, B_w_r, B_w_gate, B_w_up, B_w_down)
```

```python
import functools
import jax
import jax.numpy as jnp
from jax import lax
import jax.experimental.pallas as pl
import jax.experimental.pallas.tpu as pltpu

B, D, H, DH, SK, W, F = 4, 640, 32, 192, 4096, 1024, 1536
NC = W // 128
SCALE = DH ** -0.5
LOG2E = 1.4426950408889634
EPS = 1e-5
BF = jnp.bfloat16
F32 = jnp.float32


def _ln(x):
    m = jnp.mean(x, axis=-1, keepdims=True)
    xc = x - m
    v = jnp.mean(xc * xc, axis=-1, keepdims=True)
    return xc / jnp.sqrt(v + EPS)


def _bf(u):
    return pltpu.bitcast(u, BF)


def _u32(x):
    return pltpu.bitcast(x.astype(BF), jnp.uint32)


def default_chunks(b):
    if b < B - 1:
        return [(0, 32)], [(0, 32)]
    return [(0, 32)], [(0, 24), (24, 4), (28, 2), (30, 1), (31, 1)]


def make_kernel(isolate=True, late_issue=4, reduce_mode='mxu', scopes=False, unroll=1, chunks=default_chunks, pv_rows=16):
    KCH = [chunks(b)[0] for b in range(B)]
    VCH = [chunks(b)[1] for b in range(B)]
    ksizes = sorted({s for b in range(B) for (_, s) in KCH[b]})
    vsizes = sorted({s for b in range(B) for (_, s) in VCH[b]})

    KIDX = {}
    VIDX = {}
    for bb in range(B):
        for (h0, n) in KCH[bb]:
            KIDX[(bb, h0)] = len(KIDX)
        for (h0, n) in VCH[bb]:
            VIDX[(bb, h0)] = len(VIDX)

    def semid(is_k, b, h0):
        tab = KIDX if is_k else VIDX
        if isinstance(b, int) and isinstance(h0, int):
            return tab[(b, h0)]
        out = 0
        for (bb, hh), i in tab.items():
            if isinstance(h0, int) and hh != h0:
                continue
            out = jnp.where(jnp.logical_and(b == bb, h0 == hh), i, out)
        return out

    def scope(name):
        import contextlib
        return jax.named_scope(name) if scopes else contextlib.nullcontext()

    def _kernel(x_hbm, k_hbm, v_hbm, wq_hbm, wo_hbm, wr_hbm, wg_hbm, wu_hbm, wd_hbm,
                out_ref,
                xb, kbuf, vbuf, wq, wo_nat, wo, wr, wg, wu, wd, xs, onesb, qbuf, ilbuf, sbuf, mbuf, pbuf, lbuf, abuf, sem_w, sem_k, sem_v):
        small = [pltpu.make_async_copy(x_hbm, xb, sem_w.at[0]), pltpu.make_async_copy(wr_hbm, wr, sem_w.at[1])]
        nat = [pltpu.make_async_copy(wq_hbm, wq, sem_w.at[2]), pltpu.make_async_copy(wg_hbm, wg, sem_w.at[4]),
               pltpu.make_async_copy(wu_hbm, wu, sem_w.at[5]), pltpu.make_async_copy(wd_hbm, wd, sem_w.at[6])]

        wo_copy = pltpu.make_async_copy(wo_hbm, wo_nat, sem_w.at[3])

        def kvtile(hbm, buf, sem, b, h0, n, c):
            return pltpu.make_async_copy(hbm.at[b, pl.ds(h0, n), :, pl.ds(pl.multiple_of(SK - W + c * 128, 128), 128)],
                                         buf.at[b, pl.ds(h0, n), c], sem.at[semid(buf is kbuf, b, h0)])

        def kvall(buf, sem, b, h0, n):
            return pltpu.make_async_copy(buf.at[b, pl.ds(h0, n)], buf.at[b, pl.ds(h0, n)], sem.at[semid(buf is kbuf, b, h0)])

        def ordered(fn):
            lax.fori_loop(0, pl.num_programs(0), lambda i, c: (fn(), c)[1], 0)

        def issue_chunk(which, b, h0, n):
            def issue_kv(c, carry):
                if which == 'k':
                    kvtile(k_hbm, kbuf, sem_k, b, h0, n, c).start()
                else:
                    kvtile(v_hbm, vbuf, sem_v, b, h0, n, c).start()
                return carry
            lax.fori_loop(0, NC, issue_kv, 0)

        for c in small + nat[:1] + [wo_copy] + nat[1:]:
            c.start()
        for b in range(B):
            for (h0, n) in KCH[b]:
                issue_chunk('k', b, h0, n)
            if b < B - 1:
                for (h0, n) in VCH[b]:
                    issue_chunk('v', b, h0, n)

        small[0].wait()
        small[1].wait()
        xs[...] = jnp.zeros((8, D), F32)
        xs[0:4, :] = xb[...].astype(F32)
        wr32 = jnp.broadcast_to(wr[...].astype(F32).reshape(1, D), (8, D))
        nat[0].wait()
        wo_copy.wait()

        def retile(i, carry):
            r0 = pl.multiple_of(i * 256, 256)
            for n in range(D // 128):
                wo[n, pl.ds(r0, 256), :] = wo_nat[pl.ds(r0, 256), n * 128:(n + 1) * 128]
            return carry
        lax.fori_loop(0, H * DH // 256, retile, 0)
        for c in nat[1:]:
            c.wait()

        k32 = kbuf.bitcast(jnp.uint32)
        v32 = vbuf.bitcast(jnp.uint32)
        onesb[...] = pltpu.bitcast(jnp.ones((16, 128), BF), jnp.uint32)
        wo32 = wo.bitcast(jnp.uint32)

        LAG = 4

        def mxu_stream(jobs, after_pop=None):
            nsteps = max(len(j) for j in jobs)
            for t in range(nsteps + LAG):
                for m in range(4):
                    if 0 <= t - LAG < len(jobs[m]):
                        res = pltpu.matmul_pop_fifo((16, 128), F32, m)
                        after_pop(jobs[m][t - LAG][2], res)
                    if t < len(jobs[m]):
                        lhs, rhs_fn, _ = jobs[m][t]
                        pltpu.matmul_push_rhs(rhs_fn(), 0, m)
                        pltpu.matmul_lhs_fifo(lhs() if callable(lhs) else lhs, m, load_staged_rhs=0)

        def dup16(a):
            return jnp.concatenate([a, a], axis=0).astype(BF)

        def split128(a):
            return [a[:, i:min(i + 128, a.shape[1])] for i in range(0, a.shape[1], 128)]

        def wait_chunk(table, buf, sem, b, h, sizes):
            for s in sizes:
                cond = None
                for bb in range(B):
                    for (h0, n) in table[bb]:
                        if n != s:
                            continue
                        if isinstance(h, int):
                            if h != h0:
                                continue
                            c = b == bb
                        else:
                            c = jnp.logical_and(b == bb, h == h0)
                        cond = c if cond is None else jnp.logical_or(cond, c)
                if cond is None:
                    continue
                hh = h if isinstance(h, int) else jnp.minimum(h, H - s)
                @pl.when(cond)
                def _():
                    kvall(buf, sem, b, hh, s).wait()

        def layer_(it, carry):
            b = it // 2
            first = (it % 2) == 0

            @pl.when(it == late_issue)
            def _():
                for (h0, n) in VCH[B - 1]:
                    issue_chunk('v', B - 1, h0, n)
            x = jnp.broadcast_to(xs[pl.ds(b, 1), :], (8, D))
            xt = [dup16(a) for a in split128(_ln(x))]
            lane_q = lax.broadcasted_iota(jnp.int32, (8, 128), 1)
            lo_half = lane_q < 64
            with scope('qproj'):
                KT = D // 128
                part = {}

                def q_tile(j, t0, t1, t2):
                    r1 = pltpu.roll(t1, 64, 1)
                    r2 = pltpu.roll(t2, 64, 1)
                    qbuf[2 * j, 0] = _u32(dup16(t0))
                    qbuf[2 * j, 1] = _u32(jnp.concatenate([jnp.where(lo_half, t1, 0.0), jnp.where(lo_half, 0.0, r1)], axis=0))
                    qbuf[2 * j + 1, 0] = _u32(dup16(jnp.where(lo_half, r1, r2)))
                    qbuf[2 * j + 1, 1] = _u32(jnp.concatenate([jnp.where(lo_half, r2, 0.0), jnp.where(lo_half, 0.0, t2)], axis=0))

                def q_pop(key, res):
                    n, k = key
                    v = res[0:8]
                    part[n] = v if k == 0 else part[n] + v
                    if k == KT - 1:
                        part[n] = part[n] * (SCALE * LOG2E)
                        j = n // 3
                        if all((3 * j + t) in part and done.get(3 * j + t) for t in range(3) if 3 * j + t != n):
                            q_tile(j, part[3 * j], part[3 * j + 1], part[3 * j + 2])
                        done[n] = True
                done = {}
                jobs = [[(xt[k], (lambda n=n, k=k: wq[k * 128:(k + 1) * 128, n * 128:(n + 1) * 128]), (n, k))
                         for n in range(m, 3 * H // 2, 4) for k in range(KT)] for m in range(4)]
                mxu_stream(jobs, q_pop)

            lane = lax.broadcasted_iota(jnp.int32, (1, 128), 1)
            grp = lane // 8
            diag = (lax.broadcasted_iota(jnp.int32, (8, 128), 0) == lax.broadcasted_iota(jnp.int32, (8, 128), 1) % 8)

            def u32(x):
                return _bf(x)

            def k_rhs(h, m, j):
                if j < 2:
                    return u32(k32[b, h, 2 * m + j, 0:64, :])
                return jnp.concatenate([u32(k32[b, h, 2 * m, 64:96, :]), u32(k32[b, h, 2 * m + 1, 64:96, :])], axis=0)

            def pop(m):
                return pltpu.matmul_pop_fifo((16, 128), F32, m)


            def st_kpop(h, kres):
                ss = []
                for m in range(4):
                    f0, f1, hf = kres[m]
                    ss.append(f0[0:8] + hf[0:8])
                    ss.append(f1[0:8] + hf[8:16])
                mx = ss[0]
                for c in range(NC):
                    sbuf[h & 1, :, c * 128:(c + 1) * 128] = ss[c]
                    if c:
                        mx = jnp.maximum(mx, ss[c])
                mbuf[h & 1] = mx

            def st_soft(h):
                mx = jnp.max(mbuf[h & 1], axis=-1, keepdims=True)
                ps = None
                for c in range(NC):
                    p = jnp.exp2(sbuf[h & 1, :, c * 128:(c + 1) * 128] - mx)
                    pbuf[h & 1, :, c * 128:(c + 1) * 128] = p
                    ps = p if ps is None else ps + p
                lbuf[h & 1] = ps

            def st_b1(h):
                p = pbuf[h & 1]
                l = jnp.sum(lbuf[h & 1], axis=-1, keepdims=True)
                ilbuf[h & 3] = jnp.broadcast_to(1.0 / l, (8, 128))
                for r in range(DH // 16):
                    a0 = a1 = None
                    for c in range(NC):
                        w = v32[b, h, c, 8 * r:8 * r + 8, :]
                        pc = p[:, c * 128:(c + 1) * 128]
                        t0 = pltpu.unpack_elementwise(w, index=0, packed_dtype=BF, unpacked_dtype=F32) * pc
                        t1 = pltpu.unpack_elementwise(w, index=1, packed_dtype=BF, unpacked_dtype=F32) * pc
                        a0 = t0 if a0 is None else a0 + t0
                        a1 = t1 if a1 is None else a1 + t1
                    abuf[h & 1, 8 * r:8 * r + 8, :] = pltpu.pack_elementwise([a0, a1], packed_dtype=BF)

            def o_lhs(h, xres):
                il = ilbuf[h & 3]
                o0 = xres[0][0:8] * il
                o1 = xres[1][0:8] * il
                return [dup16(o0), jnp.concatenate([jnp.where(lo_half, o1, 0.0), jnp.where(lo_half, 0.0, o1)], axis=0).astype(BF)]

            WO_TILES = [(0,), (1,), (2,), (3,), (4,), (0, 1), (2, 3), (4, 4)]
            PROG = [[('x', 0), ('k', 0), ('k', 1), ('k', 2), ('w', 0)],
                    [('x', 1), ('k', 0), ('k', 1), ('k', 2), ('w', 1)],
                    [('k', 0), ('k', 1), ('k', 2), ('w', 2), ('w', 3), ('w', 5)],
                    [('k', 0), ('k', 1), ('k', 2), ('w', 4), ('w', 6), ('w', 7)]]

            def wo_rhs(h, t):
                r0 = pl.multiple_of(h * (DH // 2), 32) if not isinstance(h, int) else h * (DH // 2)
                t = WO_TILES[t]
                if len(t) == 1:
                    return u32(wo32[t[0], pl.ds(r0, 64), :])
                return jnp.concatenate([u32(wo32[t[0], pl.ds(r0 + 64, 32), :]), u32(wo32[t[1], pl.ds(r0 + 64, 32), :])], axis=0)

            def step(i, acc):
                static = isinstance(i, int)
                ok = (lambda h: 0 <= h < H) if static else (lambda h: True)
                hk, hkp, hs_, hb, hx, hc, hcp = i, i - 1, i - 2, i - 3, i - 4, i - 5, i - 6
                if ok(hk):
                    ql = [_bf(qbuf[hk, 0]), _bf(qbuf[hk, 1])]
                kres = [[None] * 3 for _ in range(4)]
                xres = [None, None]
                wres = [None] * 8
                ol = [None]

                def slot(m, kind, j):
                    if kind == 'k':
                        if ok(hkp):
                            kres[m][j] = pop(m)
                        if ok(hk):
                            pltpu.matmul_push_rhs(k_rhs(hk, m, j), 0, m)
                            pltpu.matmul_lhs_fifo(ql[j // 2], m, load_staged_rhs=0)
                    elif kind == 'x':
                        if ok(hc):
                            xres[j] = pop(m)
                        if ok(hx):
                            if j == 0:
                                a = _bf(abuf[hx & 1, 0:64, :])
                            else:
                                ah = _bf(abuf[hx & 1, 64:96, :])
                                a = jnp.concatenate([ah, ah], axis=0)
                            pltpu.matmul_push_rhs(a, 0, m, transpose=True)
                            pltpu.matmul_lhs_fifo(_bf(onesb[...]), m, load_staged_rhs=0)
                    else:
                        if ok(hcp):
                            wres[j] = pop(m)
                        if ok(hc):
                            if ol[0] is None:
                                ol[0] = o_lhs(hc, xres)
                            pltpu.matmul_push_rhs(wo_rhs(hc, j), 0, m)
                            pltpu.matmul_lhs_fifo(ol[0][len(WO_TILES[j]) - 1], m, load_staged_rhs=0)

                for t in range(6):
                    for m in range(4):
                        if t < len(PROG[m]):
                            slot(m, *PROG[m][t])
                if ok(hcp):
                    outs = [None] * 5
                    for j, t in enumerate(WO_TILES):
                        r = wres[j]
                        pieces = [(t[0], r[0:8])] if (len(t) == 1 or t[0] == t[1]) else [(t[0], r[0:8]), (t[1], r[8:16])]
                        for n, v in pieces:
                            outs[n] = v if outs[n] is None else outs[n] + v
                    acc = acc + jnp.concatenate(outs, axis=1)
                if ok(hb): st_b1(hb)
                if ok(hs_): st_soft(hs_)
                if ok(hkp): st_kpop(hkp, kres)
                return acc

            def vwait(h0):
                groups = {}
                for bb in range(B):
                    for (hh, n) in VCH[bb]:
                        if hh == h0:
                            groups.setdefault(n, []).append(bb)
                for n, bs in groups.items():
                    cond = first
                    if len(bs) < B:
                        c = None
                        for bb in bs:
                            c = (b == bb) if c is None else jnp.logical_or(c, b == bb)
                        cond = jnp.logical_and(first, c)
                    @pl.when(cond)
                    def _():
                        kvall(vbuf, sem_v, b, h0, n).wait()

            acc = jnp.zeros((8, D), F32)
            vstarts = sorted({h0 for bb in range(B) for (h0, n) in VCH[bb]})
            with scope('attn'):
                @pl.when(first)
                def _():
                    for (h0, n) in KCH[0]:
                        kvall(kbuf, sem_k, b, h0, n).wait()
                i = 0
                while i < H + 6:
                    if (i - 3) in vstarts:
                        vwait(i - 3)
                    nxt = min([h0 + 3 for h0 in vstarts if h0 + 3 > i] + [H])
                    if 6 <= i < H and nxt - i >= 2 * unroll:
                        cnt = (nxt - i) // unroll
                        def multi(j, acc, i0=i):
                            for u in range(unroll):
                                acc = step(i0 + j * unroll + u, acc)
                            return acc
                        acc = lax.fori_loop(0, cnt, multi, acc)
                        i += cnt * unroll
                    else:
                        if isolate:
                            acc = lax.fori_loop(0, jnp.minimum(b + 1, 1), lambda _, a, i=i: step(i, a), acc)
                        else:
                            acc = step(i, acc)
                        i += 1
            with scope('ffn'):
                x = x + acc
                xnb = _ln(x).astype(BF)
                xn32 = xnb.astype(F32)
                r = jnp.sum(xn32 * wr32, axis=-1, keepdims=True)
                xt = [dup16(a) for a in split128(xn32)]
                KT, NF, NO = D // 128, F // 128, D // 128
                gu = {}
                hs = {}
                ys = {}

                def f_pop(key, res):
                    kind, n, k = key
                    v = res[0:8]
                    if kind < 2:
                        gu[kind, n] = v if k == 0 else gu[kind, n] + v
                        if kind == 1 and k == KT - 1:
                            gt, up = gu[0, n], gu[1, n]
                            hs[n] = dup16(gt * jax.nn.sigmoid(gt) * up)
                    else:
                        ys[n] = v if n not in ys else ys[n] + v
                jobs = []
                for m in range(4):
                    jm = []
                    for n in range(m, NF, 4):
                        for kind, w in ((0, wg), (1, wu)):
                            for k in range(KT):
                                jm.append((xt[k], (lambda w=w, n=n, k=k: w[k * 128:(k + 1) * 128, n * 128:(n + 1) * 128]), (kind, n, k)))
                    for k in range(m, NF, 4):
                        for n in range(NO):
                            jm.append(((lambda k=k: hs[k]), (lambda n=n, k=k: wd[k * 128:(k + 1) * 128, n * 128:(n + 1) * 128]), (2, n, k)))
                    jobs.append(jm)
                mxu_stream(jobs, f_pop)
                y = jnp.concatenate([ys[n] for n in range(NO)], axis=1)
                y = y * jax.nn.sigmoid(r)
                x = x + (xn32 + (xn32 * 0.0 + y))
                xs[pl.ds(b, 1), :] = x[0:1, :]
            return carry

        def layer(it, carry):
            with scope('layer'):
                return layer_(it, carry)

        lax.fori_loop(0, 2 * B, layer, 0)
        out_ref[...] = xs[0:4, :].astype(BF)

    @jax.jit
    def kernel_fn(A_x, A_k_cache, A_v_cache, A_wq, A_wo, B_x, B_w_r, B_w_gate, B_w_up, B_w_down):
        kt = jnp.swapaxes(A_k_cache, 2, 3)
        vt = jnp.swapaxes(A_v_cache, 2, 3)
        x2 = A_x.reshape(B, D)
        anyspec = pl.BlockSpec(memory_space=pl.ANY)
        out = pl.pallas_call(
            _kernel,
            out_shape=jax.ShapeDtypeStruct((B, D), BF), grid=(1,),
            in_specs=[anyspec] * 9,
            out_specs=pl.BlockSpec(memory_space=pltpu.VMEM),
            scratch_shapes=[
                pltpu.VMEM((B, D), BF),
                pltpu.VMEM((B, H, NC, DH, 128), BF),
                pltpu.VMEM((B, H, NC, DH, 128), BF),
                pltpu.VMEM((D, H * DH), BF),
                pltpu.VMEM((H * DH, D), BF),
                pltpu.VMEM((D // 128, H * DH, 128), BF),
                pltpu.VMEM((D,), BF),
                pltpu.VMEM((D, F), BF),
                pltpu.VMEM((D, F), BF),
                pltpu.VMEM((F, D), BF),
                pltpu.VMEM((8, D), F32),
                pltpu.VMEM((8, 128), jnp.uint32),
                pltpu.VMEM((H, 2, 8, 128), jnp.uint32),
                pltpu.VMEM((4, 8, 128), F32),
                pltpu.VMEM((2, 8, W), F32),
                pltpu.VMEM((2, 8, 128), F32),
                pltpu.VMEM((2, 8, W), F32),
                pltpu.VMEM((2, 8, 128), F32),
                pltpu.VMEM((2, DH // 2, 128), jnp.uint32),
                pltpu.SemaphoreType.DMA((7,)),
                pltpu.SemaphoreType.DMA((len(KIDX),)),
                pltpu.SemaphoreType.DMA((len(VIDX),)),
            ],
            compiler_params=pltpu.CompilerParams(vmem_limit_bytes=127 * 1024 * 1024),
        )(x2, kt, vt, A_wq, A_wo, B_w_r, B_w_gate, B_w_up, B_w_down)
        return out.reshape(B, 1, D)
    return kernel_fn


_impl = make_kernel()


@jax.jit
def pallas_interleave_layers__sliding_block_cached__moe_arch_mod__decode_kernel(
    A_x, A_k_cache, A_v_cache, A_wq, A_wo, B_x, B_w_r, B_w_gate, B_w_up, B_w_down
):
    return _impl(A_x, A_k_cache, A_v_cache, A_wq, A_wo, B_x, B_w_r, B_w_gate, B_w_up, B_w_down)
```

```python
import functools
import jax
import jax.numpy as jnp
from jax import lax
import jax.experimental.pallas as pl
import jax.experimental.pallas.tpu as pltpu

B, D, H, DH, SK, W, F = 4, 640, 32, 192, 4096, 1024, 1536
NC = W // 128
SCALE = DH ** -0.5
LOG2E = 1.4426950408889634
EPS = 1e-5
BF = jnp.bfloat16
F32 = jnp.float32


def _ln(x):
    t = [x[:, i:i + 128] for i in range(0, x.shape[1], 128)]
    s1 = functools.reduce(jnp.add, t)
    s2 = functools.reduce(jnp.add, [a * a for a in t])
    n = x.shape[1]
    m = jnp.sum(s1, axis=-1, keepdims=True) * (1.0 / n)
    q = jnp.sum(s2, axis=-1, keepdims=True) * (1.0 / n)
    v = jnp.maximum(q - m * m, 0.0)
    return (x - m) * lax.rsqrt(v + EPS)


def _bf(u):
    return pltpu.bitcast(u, BF)


def _u32(x):
    return pltpu.bitcast(x.astype(BF), jnp.uint32)


def default_chunks(b):
    if b < B - 1:
        return [(0, 32)], [(0, 32)]
    return [(0, 32)], [(0, 24), (24, 4), (28, 2), (30, 1), (31, 1)]


def make_kernel(noh=True, prog=None, order='mfbsk', morder=(0, 1, 2, 3), slot_major=True, split=None, acc_mem=True, late_pop=True, flat=True, iso_from=3, isolate=False, late_issue=4, reduce_mode='mxu', scopes=False, unroll=1, chunks=default_chunks, pv_rows=16):
    KCH = [chunks(b)[0] for b in range(B)]
    VCH = [chunks(b)[1] for b in range(B)]
    ksizes = sorted({s for b in range(B) for (_, s) in KCH[b]})
    vsizes = sorted({s for b in range(B) for (_, s) in VCH[b]})

    KIDX = {}
    VIDX = {}
    for bb in range(B):
        for (h0, n) in KCH[bb]:
            KIDX[(bb, h0)] = len(KIDX)
        for (h0, n) in VCH[bb]:
            VIDX[(bb, h0)] = len(VIDX)

    def semid(is_k, b, h0):
        tab = KIDX if is_k else VIDX
        if isinstance(b, int) and isinstance(h0, int):
            return tab[(b, h0)]
        out = 0
        for (bb, hh), i in tab.items():
            if isinstance(h0, int) and hh != h0:
                continue
            out = jnp.where(jnp.logical_and(b == bb, h0 == hh), i, out)
        return out

    def scope(name):
        import contextlib
        return jax.named_scope(name) if scopes else contextlib.nullcontext()

    def _kernel(x_hbm, k_hbm, v_hbm, wq_hbm, wo_hbm, wr_hbm, wg_hbm, wu_hbm, wd_hbm,
                out_ref,
                xb, kbuf, vbuf, wq, wo_nat, wo, wr, wg, wu, wd, xs, accb, onesb, qbuf, ilbuf, sbuf, mbuf, pbuf, lbuf, abuf, sem_w, sem_k, sem_v):
        small = [pltpu.make_async_copy(x_hbm, xb, sem_w.at[0]), pltpu.make_async_copy(wr_hbm, wr, sem_w.at[1])]
        nat = [pltpu.make_async_copy(wq_hbm, wq, sem_w.at[2]), pltpu.make_async_copy(wg_hbm, wg, sem_w.at[4]),
               pltpu.make_async_copy(wu_hbm, wu, sem_w.at[5]), pltpu.make_async_copy(wd_hbm, wd, sem_w.at[6])]

        wo_copy = pltpu.make_async_copy(wo_hbm, wo_nat, sem_w.at[3])

        def kvtile(hbm, buf, sem, b, h0, n, c):
            return pltpu.make_async_copy(hbm.at[b, pl.ds(h0, n), :, pl.ds(pl.multiple_of(SK - W + c * 128, 128), 128)],
                                         buf.at[pl.ds(b * H + h0, n), c], sem.at[semid(buf is kbuf, b, h0)])

        def kvall(buf, sem, b, h0, n):
            return pltpu.make_async_copy(buf.at[pl.ds(b * H + h0, n)], buf.at[pl.ds(b * H + h0, n)], sem.at[semid(buf is kbuf, b, h0)])

        def ordered(fn):
            lax.fori_loop(0, pl.num_programs(0), lambda i, c: (fn(), c)[1], 0)

        def issue_chunk(which, b, h0, n):
            def issue_kv(c, carry):
                if which == 'k':
                    kvtile(k_hbm, kbuf, sem_k, b, h0, n, c).start()
                else:
                    kvtile(v_hbm, vbuf, sem_v, b, h0, n, c).start()
                return carry
            lax.fori_loop(0, NC, issue_kv, 0)

        for c in small + nat[:1] + [wo_copy] + nat[1:]:
            c.start()
        for b in range(B):
            for (h0, n) in KCH[b]:
                issue_chunk('k', b, h0, n)
            if b < B - 1:
                for (h0, n) in VCH[b]:
                    issue_chunk('v', b, h0, n)

        small[0].wait()
        small[1].wait()
        xs[...] = jnp.zeros((8, D), F32)
        xs[0:4, :] = xb[...].astype(F32)
        wr32 = jnp.broadcast_to(wr[...].astype(F32).reshape(1, D), (8, D))
        nat[0].wait()
        wo_copy.wait()

        def retile(i, carry):
            r0 = pl.multiple_of(i * 256, 256)
            for n in range(D // 128):
                wo[n, pl.ds(r0, 256), :] = wo_nat[pl.ds(r0, 256), n * 128:(n + 1) * 128]
            return carry
        lax.fori_loop(0, H * DH // 256, retile, 0)
        for c in nat[1:]:
            c.wait()

        if noh:
            sbuf, mbuf, pbuf, lbuf, abuf, ilbuf = [pltpu.annotate(r, no_hazard=True) for r in (sbuf, mbuf, pbuf, lbuf, abuf, ilbuf)]
        k32 = kbuf.bitcast(jnp.uint32)
        v32 = vbuf.bitcast(jnp.uint32)
        onesb[...] = pltpu.bitcast(jnp.ones((16, 128), BF), jnp.uint32)
        wo32 = wo.bitcast(jnp.uint32)

        LAG = 4

        def mxu_stream(jobs, after_pop=None):
            nsteps = max(len(j) for j in jobs)
            for t in range(nsteps + LAG):
                for m in range(4):
                    if 0 <= t - LAG < len(jobs[m]):
                        res = pltpu.matmul_pop_fifo((16, 128), F32, m)
                        after_pop(jobs[m][t - LAG][2], res)
                    if t < len(jobs[m]):
                        lhs, rhs_fn, _ = jobs[m][t]
                        pltpu.matmul_push_rhs(rhs_fn(), 0, m)
                        pltpu.matmul_lhs_fifo(lhs() if callable(lhs) else lhs, m, load_staged_rhs=0)

        def dup16(a):
            return jnp.concatenate([a, a], axis=0).astype(BF)

        def split128(a):
            return [a[:, i:min(i + 128, a.shape[1])] for i in range(0, a.shape[1], 128)]

        def wait_chunk(table, buf, sem, b, h, sizes):
            for s in sizes:
                cond = None
                for bb in range(B):
                    for (h0, n) in table[bb]:
                        if n != s:
                            continue
                        if isinstance(h, int):
                            if h != h0:
                                continue
                            c = b == bb
                        else:
                            c = jnp.logical_and(b == bb, h == h0)
                        cond = c if cond is None else jnp.logical_or(cond, c)
                if cond is None:
                    continue
                hh = h if isinstance(h, int) else jnp.minimum(h, H - s)
                @pl.when(cond)
                def _():
                    kvall(buf, sem, b, hh, s).wait()

        def layer_(it, carry):
            b = it // 2
            first = (it % 2) == 0

            @pl.when(it == late_issue)
            def _():
                for (h0, n) in VCH[B - 1]:
                    issue_chunk('v', B - 1, h0, n)
            @pl.when(first)
            def _():
                for (h0, n) in KCH[0]:
                    kvall(kbuf, sem_k, b, h0, n).wait()
            x = jnp.broadcast_to(xs[pl.ds(b, 1), :], (8, D))
            xt = [dup16(a) for a in split128(_ln(x))]
            lane_q = lax.broadcasted_iota(jnp.int32, (8, 128), 1)
            lo_half = lane_q < 64
            with scope('qproj'):
                KT = D // 128
                part = {}

                def q_tile(j, t0, t1, t2):
                    r1 = pltpu.roll(t1, 64, 1)
                    r2 = pltpu.roll(t2, 64, 1)
                    qbuf[2 * j, 0] = _u32(dup16(t0))
                    qbuf[2 * j, 1] = _u32(jnp.concatenate([jnp.where(lo_half, t1, 0.0), jnp.where(lo_half, 0.0, r1)], axis=0))
                    qbuf[2 * j + 1, 0] = _u32(dup16(jnp.where(lo_half, r1, r2)))
                    qbuf[2 * j + 1, 1] = _u32(jnp.concatenate([jnp.where(lo_half, r2, 0.0), jnp.where(lo_half, 0.0, t2)], axis=0))

                def q_pop(key, res):
                    n, k = key
                    v = res[0:8]
                    part[n] = v if k == 0 else part[n] + v
                    if k == KT - 1:
                        part[n] = part[n] * (SCALE * LOG2E)
                        j = n // 3
                        if all((3 * j + t) in part and done.get(3 * j + t) for t in range(3) if 3 * j + t != n):
                            q_tile(j, part[3 * j], part[3 * j + 1], part[3 * j + 2])
                        done[n] = True
                done = {}
                jobs = [[(xt[k], (lambda n=n, k=k: wq[k * 128:(k + 1) * 128, n * 128:(n + 1) * 128]), (n, k))
                         for n in range(m, 3 * H // 2, 4) for k in range(KT)] for m in range(4)]
                mxu_stream(jobs, q_pop)

            lane = lax.broadcasted_iota(jnp.int32, (1, 128), 1)
            grp = lane // 8
            diag = (lax.broadcasted_iota(jnp.int32, (8, 128), 0) == lax.broadcasted_iota(jnp.int32, (8, 128), 1) % 8)

            def u32(x):
                return _bf(x)

            def k_rhs(h, m, j):
                if j < 2:
                    return u32(k32[b * H + h, 2 * m + j, 0:64, :])
                return jnp.concatenate([u32(k32[b * H + h, 2 * m, 64:96, :]), u32(k32[b * H + h, 2 * m + 1, 64:96, :])], axis=0)

            def pop(m):
                return pltpu.matmul_pop_fifo((16, 128), F32, m)


            def st_kpop(h, kres):
                ss = []
                for m in range(4):
                    f0, f1, hf = kres[m]
                    ss.append(f0[0:8] + hf[0:8])
                    ss.append(f1[0:8] + hf[8:16])
                mx = ss[0]
                for c in range(NC):
                    sbuf[h & 1, :, c * 128:(c + 1) * 128] = ss[c]
                    if c:
                        mx = jnp.maximum(mx, ss[c])
                mbuf[h & 1] = mx

            def st_soft(h):
                mx = jnp.max(mbuf[h & 1], axis=-1, keepdims=True)
                ps = None
                for c in range(NC):
                    p = jnp.exp2(sbuf[h & 1, :, c * 128:(c + 1) * 128] - mx)
                    pbuf[h & 1, :, c * 128:(c + 1) * 128] = p
                    ps = p if ps is None else ps + p
                lbuf[h & 1] = ps

            def st_b1(h, lo=0, hi=DH // 16, do_l=True):
                p = pbuf[h & 1]
                if do_l:
                    l = jnp.sum(lbuf[h & 1], axis=-1, keepdims=True)
                    ilbuf[h & 3] = jnp.broadcast_to(1.0 / l, (8, 128))
                for r in range(lo, hi):
                    a0 = a1 = None
                    for c in range(NC):
                        w = v32[b * H + h, c, 8 * r:8 * r + 8, :]
                        pc = p[:, c * 128:(c + 1) * 128]
                        t0 = pltpu.unpack_elementwise(w, index=0, packed_dtype=BF, unpacked_dtype=F32) * pc
                        t1 = pltpu.unpack_elementwise(w, index=1, packed_dtype=BF, unpacked_dtype=F32) * pc
                        a0 = t0 if a0 is None else a0 + t0
                        a1 = t1 if a1 is None else a1 + t1
                    abuf[h & 1, 8 * r:8 * r + 8, :] = pltpu.pack_elementwise([a0, a1], packed_dtype=BF)

            def o_lhs(h, xres):
                il = ilbuf[h & 3]
                o0 = xres[0][0:8] * il
                o1 = xres[1][0:8] * il
                return [dup16(o0), jnp.concatenate([jnp.where(lo_half, o1, 0.0), jnp.where(lo_half, 0.0, o1)], axis=0).astype(BF)]

            WO_TILES = [(0,), (1,), (2,), (3,), (4,), (0, 1), (2, 3), (4, 4)]
            PROG = prog or [[('x', 0), ('k', 0), ('k', 1), ('k', 2), ('w', 0)],
                            [('x', 1), ('k', 0), ('k', 1), ('k', 2), ('w', 1)],
                            [('k', 0), ('k', 1), ('k', 2), ('w', 2), ('w', 3), ('w', 5)],
                            [('k', 0), ('k', 1), ('k', 2), ('w', 4), ('w', 6), ('w', 7)]]

            def wo_rhs(h, t):
                r0 = pl.multiple_of(h * (DH // 2), 32) if not isinstance(h, int) else h * (DH // 2)
                t = WO_TILES[t]
                if len(t) == 1:
                    return u32(wo32[t[0], pl.ds(r0, 64), :])
                return jnp.concatenate([u32(wo32[t[0], pl.ds(r0 + 64, 32), :]), u32(wo32[t[1], pl.ds(r0 + 64, 32), :])], axis=0)

            def step(i, acc):
                static = isinstance(i, int)
                ok = (lambda h: 0 <= h < H) if static else (lambda h: True)
                hk, hkp, hs_, hb, hx, hc, hcp = i, i - 1, i - 2, i - 3, i - 4, i - 5, i - 6
                if ok(hk):
                    ql = [_bf(qbuf[hk, 0]), _bf(qbuf[hk, 1])]
                kres = [[None] * 3 for _ in range(4)]
                xres = [None, None]
                wres = [None] * 8
                ol = [None]

                def slot(m, kind, j):
                    if kind == 'k':
                        if ok(hkp) and not late_pop:
                            kres[m][j] = pop(m)
                        if ok(hk):
                            pltpu.matmul_push_rhs(k_rhs(hk, m, j), 0, m)
                            pltpu.matmul_lhs_fifo(ql[j // 2], m, load_staged_rhs=0)
                        if ok(hkp) and late_pop:
                            kres[m][j] = pop(m)
                    elif kind == 'x':
                        if ok(hc):
                            xres[j] = pop(m)
                        if ok(hx):
                            if j == 0:
                                a = _bf(abuf[hx & 1, 0:64, :])
                            else:
                                ah = _bf(abuf[hx & 1, 64:96, :])
                                a = jnp.concatenate([ah, ah], axis=0)
                            pltpu.matmul_push_rhs(a, 0, m, transpose=True)
                            pltpu.matmul_lhs_fifo(_bf(onesb[...]), m, load_staged_rhs=0)
                    else:
                        if ok(hcp) and not late_pop:
                            wres[j] = pop(m)
                        if ok(hc):
                            if ol[0] is None:
                                ol[0] = o_lhs(hc, xres)
                            pltpu.matmul_push_rhs(wo_rhs(hc, j), 0, m)
                            pltpu.matmul_lhs_fifo(ol[0][len(WO_TILES[j]) - 1], m, load_staged_rhs=0)
                        if ok(hcp) and late_pop:
                            wres[j] = pop(m)

                def part(t0, t1, g0, g1, tail):
                    for t in range(t0, t1):
                        for m in range(4):
                            if t < len(PROG[m]):
                                slot(m, *PROG[m][t])
                    if ok(hb): st_b1(hb, g0, g1, do_l=(g0 == 0))

                def fin(acc):
                    if ok(hcp):
                        outs = [None] * 5
                        for j, t in enumerate(WO_TILES):
                            r = wres[j]
                            pieces = [(t[0], r[0:8])] if (len(t) == 1 or t[0] == t[1]) else [(t[0], r[0:8]), (t[1], r[8:16])]
                            for n, v in pieces:
                                outs[n] = v if outs[n] is None else outs[n] + v
                        if acc_mem:
                            accb[...] = accb[...] + jnp.concatenate(outs, axis=1)
                        else:
                            acc = acc + jnp.concatenate(outs, axis=1)
                    return acc

                if split and not static:
                    bounds = split
                    prev_t, prev_g = 0, 0
                    for idx, (t1, g1) in enumerate(bounds):
                        if idx == 0:
                            part(prev_t, t1, prev_g, g1, False)
                            if ok(hs_): st_soft(hs_)
                        else:
                            def blk(_, c, a=prev_t, t1=t1, g0=prev_g, g1=g1, last=(idx == len(bounds) - 1)):
                                part(a, t1, g0, g1, last)
                                if last:
                                    fin(0)
                                    if ok(hkp): st_kpop(hkp, kres)
                                return c
                            lax.fori_loop(0, jnp.minimum(b + 1, 1), blk, 0)
                        prev_t, prev_g = t1, g1
                    return acc
                def mx():
                    if slot_major:
                        for t in range(6):
                            for m in morder:
                                if t < len(PROG[m]):
                                    slot(m, *PROG[m][t])
                    else:
                        tm = [0] * 4
                        pos = [0] * 4
                        while any(pos[m] < len(PROG[m]) for m in range(4)):
                            cand = [m for m in morder if pos[m] < len(PROG[m])]
                            m = min(cand, key=lambda q: tm[q])
                            slot(m, *PROG[m][pos[m]])
                            tm[m] += 2 if PROG[m][pos[m]][0] == 'x' else 1
                            pos[m] += 1
                for what in order:
                    if what == 'm': mx()
                    elif what == 'b' and ok(hb): st_b1(hb)
                    elif what == 'f': acc = fin(acc)
                    elif what == 's' and ok(hs_): st_soft(hs_)
                    elif what == 'k' and ok(hkp): st_kpop(hkp, kres)
                return acc

            def vwait(h0):
                groups = {}
                for bb in range(B):
                    for (hh, n) in VCH[bb]:
                        if hh == h0:
                            groups.setdefault(n, []).append(bb)
                for n, bs in groups.items():
                    cond = first
                    if len(bs) < B:
                        c = None
                        for bb in bs:
                            c = (b == bb) if c is None else jnp.logical_or(c, b == bb)
                        cond = jnp.logical_and(first, c)
                    @pl.when(cond)
                    def _():
                        kvall(vbuf, sem_v, b, h0, n).wait()

            if acc_mem:
                accb[...] = jnp.zeros((8, D), F32)
                acc = 0
            else:
                acc = jnp.zeros((8, D), F32)
            vstarts = sorted({h0 for bb in range(B) for (h0, n) in VCH[bb]})
            with scope('attn'):
                i = 0
                while i < H + 6:
                    if (i - 3) in vstarts:
                        vwait(i - 3)
                    nxt = min([h0 + 3 for h0 in vstarts if h0 + 3 > i] + [H])
                    if 6 <= i < H and nxt - i >= 2 * unroll:
                        cnt = (nxt - i) // unroll
                        def multi(j, acc, i0=i):
                            for u in range(unroll):
                                acc = step(i0 + j * unroll + u, acc)
                            return acc
                        acc = lax.fori_loop(0, cnt, multi, acc)
                        i += cnt * unroll
                    else:
                        if isolate and i >= iso_from:
                            acc = lax.fori_loop(0, jnp.minimum(b + 1, 1), lambda _, a, i=i: step(i, a), acc)
                        else:
                            acc = step(i, acc)
                        i += 1
            with scope('ffn'):
                x = x + (accb[...] if acc_mem else acc)
                xnb = _ln(x).astype(BF)
                xn32 = xnb.astype(F32)
                r = jnp.sum(xn32 * wr32, axis=-1, keepdims=True)
                xt = [dup16(a) for a in split128(xn32)]
                KT, NF, NO = D // 128, F // 128, D // 128
                gu = {}
                hs = {}
                ys = {}

                def f_pop(key, res):
                    kind, n, k = key
                    v = res[0:8]
                    if kind < 2:
                        gu[kind, n] = v if k == 0 else gu[kind, n] + v
                        if kind == 1 and k == KT - 1:
                            gt, up = gu[0, n], gu[1, n]
                            hs[n] = dup16(gt * jax.nn.sigmoid(gt) * up)
                    else:
                        ys[n] = v if n not in ys else ys[n] + v
                jobs = []
                for m in range(4):
                    jm = []
                    for n in range(m, NF, 4):
                        for kind, w in ((0, wg), (1, wu)):
                            for k in range(KT):
                                jm.append((xt[k], (lambda w=w, n=n, k=k: w[k * 128:(k + 1) * 128, n * 128:(n + 1) * 128]), (kind, n, k)))
                    for k in range(m, NF, 4):
                        for n in range(NO):
                            jm.append(((lambda k=k: hs[k]), (lambda n=n, k=k: wd[k * 128:(k + 1) * 128, n * 128:(n + 1) * 128]), (2, n, k)))
                    jobs.append(jm)
                mxu_stream(jobs, f_pop)
                y = jnp.concatenate([ys[n] for n in range(NO)], axis=1)
                y = y * jax.nn.sigmoid(r)
                x = x + (xn32 + (xn32 * 0.0 + y))
                xs[pl.ds(b, 1), :] = x[0:1, :]
            return carry

        def layer(it, carry):
            with scope('layer'):
                return layer_(it, carry)

        lax.fori_loop(0, 2 * B, layer, 0)
        out_ref[...] = xs[0:4, :].astype(BF)

    @jax.jit
    def kernel_fn(A_x, A_k_cache, A_v_cache, A_wq, A_wo, B_x, B_w_r, B_w_gate, B_w_up, B_w_down):
        kt = jnp.swapaxes(A_k_cache, 2, 3)
        vt = jnp.swapaxes(A_v_cache, 2, 3)
        x2 = A_x.reshape(B, D)
        anyspec = pl.BlockSpec(memory_space=pl.ANY)
        out = pl.pallas_call(
            _kernel,
            out_shape=jax.ShapeDtypeStruct((B, D), BF), grid=(1,),
            in_specs=[anyspec] * 9,
            out_specs=pl.BlockSpec(memory_space=pltpu.VMEM),
            scratch_shapes=[
                pltpu.VMEM((B, D), BF),
                pltpu.VMEM((B * H, NC, DH, 128), BF),
                pltpu.VMEM((B * H, NC, DH, 128), BF),
                pltpu.VMEM((D, H * DH), BF),
                pltpu.VMEM((H * DH, D), BF),
                pltpu.VMEM((D // 128, H * DH, 128), BF),
                pltpu.VMEM((D,), BF),
                pltpu.VMEM((D, F), BF),
                pltpu.VMEM((D, F), BF),
                pltpu.VMEM((F, D), BF),
                pltpu.VMEM((8, D), F32),
                pltpu.VMEM((8, D), F32),
                pltpu.VMEM((8, 128), jnp.uint32),
                pltpu.VMEM((H, 2, 8, 128), jnp.uint32),
                pltpu.VMEM((4, 8, 128), F32),
                pltpu.VMEM((2, 8, W), F32),
                pltpu.VMEM((2, 8, 128), F32),
                pltpu.VMEM((2, 8, W), F32),
                pltpu.VMEM((2, 8, 128), F32),
                pltpu.VMEM((2, DH // 2, 128), jnp.uint32),
                pltpu.SemaphoreType.DMA((7,)),
                pltpu.SemaphoreType.DMA((len(KIDX),)),
                pltpu.SemaphoreType.DMA((len(VIDX),)),
            ],
            compiler_params=pltpu.CompilerParams(vmem_limit_bytes=127 * 1024 * 1024),
        )(x2, kt, vt, A_wq, A_wo, B_w_r, B_w_gate, B_w_up, B_w_down)
        return out.reshape(B, 1, D)
    return kernel_fn


_impl = make_kernel()


@jax.jit
def pallas_interleave_layers__sliding_block_cached__moe_arch_mod__decode_kernel(
    A_x, A_k_cache, A_v_cache, A_wq, A_wo, B_x, B_w_r, B_w_gate, B_w_up, B_w_down
):
    return _impl(A_x, A_k_cache, A_v_cache, A_wq, A_wo, B_x, B_w_r, B_w_gate, B_w_up, B_w_down)
```

```python
import functools
import jax
import jax.numpy as jnp
from jax import lax
import jax.experimental.pallas as pl
import jax.experimental.pallas.tpu as pltpu

B, D, H, DH, SK, W, F = 4, 640, 32, 192, 4096, 1024, 1536
NC = W // 128
SCALE = DH ** -0.5
LOG2E = 1.4426950408889634
EPS = 1e-5
BF = jnp.bfloat16
F32 = jnp.float32


def _ln(x):
    t = [x[:, i:i + 128] for i in range(0, x.shape[1], 128)]
    s1 = functools.reduce(jnp.add, t)
    s2 = functools.reduce(jnp.add, [a * a for a in t])
    n = x.shape[1]
    m = jnp.sum(s1, axis=-1, keepdims=True) * (1.0 / n)
    q = jnp.sum(s2, axis=-1, keepdims=True) * (1.0 / n)
    v = jnp.maximum(q - m * m, 0.0)
    return (x - m) * lax.rsqrt(v + EPS)


def _ln_stats(x):
    t = [x[:, i:i + 128] for i in range(0, x.shape[1], 128)]
    s1 = functools.reduce(jnp.add, t)
    s2 = functools.reduce(jnp.add, [a * a for a in t])
    n = x.shape[1]
    m = jnp.sum(s1, axis=-1, keepdims=True) * (1.0 / n)
    q = jnp.sum(s2, axis=-1, keepdims=True) * (1.0 / n)
    v = jnp.maximum(q - m * m, 0.0)
    return m, lax.rsqrt(v + EPS)


def _bf(u):
    return pltpu.bitcast(u, BF)


def _u32(x):
    return pltpu.bitcast(x.astype(BF), jnp.uint32)


V3 = [(0, 16), (16, 8), (24, 4), (28, 2), (30, 1), (31, 1)]


def default_chunks(b):
    if b < B - 1:
        return [(0, 32)], [(0, 32)]
    return [(0, 32)], V3


def make_kernel(noh=True, prog=None, order='mfbsk', morder=(0, 1, 2, 3), slot_major=True, split=None, acc_mem=True, late_pop=True, flat=True, iso_from=30, isolate=True, late_issue=4, reduce_mode='mxu', scopes=False, unroll=1, chunks=default_chunks, pv_rows=16):
    KCH = [chunks(b)[0] for b in range(B)]
    VCH = [chunks(b)[1] for b in range(B)]
    ksizes = sorted({s for b in range(B) for (_, s) in KCH[b]})
    vsizes = sorted({s for b in range(B) for (_, s) in VCH[b]})

    KIDX = {}
    VIDX = {}
    for bb in range(B):
        for (h0, n) in KCH[bb]:
            KIDX[(bb, h0)] = len(KIDX)
        for (h0, n) in VCH[bb]:
            VIDX[(bb, h0)] = len(VIDX)

    def semid(is_k, b, h0):
        tab = KIDX if is_k else VIDX
        if isinstance(b, int) and isinstance(h0, int):
            return tab[(b, h0)]
        out = 0
        for (bb, hh), i in tab.items():
            if isinstance(h0, int) and hh != h0:
                continue
            out = jnp.where(jnp.logical_and(b == bb, h0 == hh), i, out)
        return out

    def scope(name):
        import contextlib
        return jax.named_scope(name) if scopes else contextlib.nullcontext()

    def _kernel(x_hbm, k_hbm, v_hbm, wq_hbm, wo_hbm, wr_hbm, wg_hbm, wu_hbm, wd_hbm,
                out_ref,
                xb, kbuf, vbuf, wq, wo_nat, wo, wr, wg, wu, wd, xs, accb, onesb, qbuf, ilbuf, sbuf, mbuf, pbuf, lbuf, abuf, sem_w, sem_k, sem_v):
        small = [pltpu.make_async_copy(x_hbm, xb, sem_w.at[0]), pltpu.make_async_copy(wr_hbm, wr, sem_w.at[1])]
        nat = [pltpu.make_async_copy(wq_hbm, wq, sem_w.at[2]), pltpu.make_async_copy(wg_hbm, wg, sem_w.at[4]),
               pltpu.make_async_copy(wu_hbm, wu, sem_w.at[5]), pltpu.make_async_copy(wd_hbm, wd, sem_w.at[6])]

        wo_copy = pltpu.make_async_copy(wo_hbm, wo_nat, sem_w.at[3])

        def kvtile(hbm, buf, sem, b, h0, n, c):
            return pltpu.make_async_copy(hbm.at[b, pl.ds(h0, n), :, pl.ds(pl.multiple_of(SK - W + c * 128, 128), 128)],
                                         buf.at[pl.ds(b * H + h0, n), c], sem.at[semid(buf is kbuf, b, h0)])

        def kvall(buf, sem, b, h0, n):
            return pltpu.make_async_copy(buf.at[pl.ds(b * H + h0, n)], buf.at[pl.ds(b * H + h0, n)], sem.at[semid(buf is kbuf, b, h0)])

        def ordered(fn):
            lax.fori_loop(0, pl.num_programs(0), lambda i, c: (fn(), c)[1], 0)

        def issue_chunk(which, b, h0, n):
            def issue_kv(c, carry):
                if which == 'k':
                    kvtile(k_hbm, kbuf, sem_k, b, h0, n, c).start()
                else:
                    kvtile(v_hbm, vbuf, sem_v, b, h0, n, c).start()
                return carry
            lax.fori_loop(0, NC, issue_kv, 0)

        for c in small + nat[:1] + [wo_copy] + nat[1:]:
            c.start()
        for b in range(B):
            for (h0, n) in KCH[b]:
                issue_chunk('k', b, h0, n)
            if b < B - 1:
                for (h0, n) in VCH[b]:
                    issue_chunk('v', b, h0, n)

        small[0].wait()
        small[1].wait()
        xs[...] = jnp.zeros((8, D), F32)
        xs[0:4, :] = xb[...].astype(F32)
        wr32 = jnp.broadcast_to(wr[...].astype(F32).reshape(1, D), (8, D))
        nat[0].wait()
        wo_copy.wait()

        def retile(i, carry):
            r0 = pl.multiple_of(i * 256, 256)
            for n in range(D // 128):
                wo[n, pl.ds(r0, 256), :] = wo_nat[pl.ds(r0, 256), n * 128:(n + 1) * 128]
            return carry
        lax.fori_loop(0, H * DH // 256, retile, 0)
        for c in nat[1:]:
            c.wait()

        if noh:
            sbuf, mbuf, pbuf, lbuf, abuf, ilbuf = [pltpu.annotate(r, no_hazard=True) for r in (sbuf, mbuf, pbuf, lbuf, abuf, ilbuf)]
        k32 = kbuf.bitcast(jnp.uint32)
        v32 = vbuf.bitcast(jnp.uint32)
        onesb[...] = pltpu.bitcast(jnp.ones((16, 128), BF), jnp.uint32)
        wo32 = wo.bitcast(jnp.uint32)

        LAG = 4

        def mxu_stream(jobs, after_pop=None):
            nsteps = max(len(j) for j in jobs)
            for t in range(nsteps + LAG):
                for m in range(4):
                    if 0 <= t - LAG < len(jobs[m]):
                        res = pltpu.matmul_pop_fifo((16, 128), F32, m)
                        after_pop(jobs[m][t - LAG][2], res)
                    if t < len(jobs[m]):
                        lhs, rhs_fn, _ = jobs[m][t]
                        pltpu.matmul_push_rhs(rhs_fn(), 0, m)
                        pltpu.matmul_lhs_fifo(lhs() if callable(lhs) else lhs, m, load_staged_rhs=0)

        def with_ones(a):
            return jnp.concatenate([a, jnp.ones_like(a)], axis=0).astype(BF)

        def dup16(a):
            return jnp.concatenate([a, a], axis=0).astype(BF)

        def split128(a):
            return [a[:, i:min(i + 128, a.shape[1])] for i in range(0, a.shape[1], 128)]

        def wait_chunk(table, buf, sem, b, h, sizes):
            for s in sizes:
                cond = None
                for bb in range(B):
                    for (h0, n) in table[bb]:
                        if n != s:
                            continue
                        if isinstance(h, int):
                            if h != h0:
                                continue
                            c = b == bb
                        else:
                            c = jnp.logical_and(b == bb, h == h0)
                        cond = c if cond is None else jnp.logical_or(cond, c)
                if cond is None:
                    continue
                hh = h if isinstance(h, int) else jnp.minimum(h, H - s)
                @pl.when(cond)
                def _():
                    kvall(buf, sem, b, hh, s).wait()

        def layer_(it, carry):
            b = it // 2
            first = (it % 2) == 0

            @pl.when(it == late_issue)
            def _():
                for (h0, n) in VCH[B - 1]:
                    issue_chunk('v', B - 1, h0, n)
            @pl.when(first)
            def _():
                for (h0, n) in KCH[0]:
                    kvall(kbuf, sem_k, b, h0, n).wait()
            x = jnp.broadcast_to(xs[pl.ds(b, 1), :], (8, D))
            m_, rs_ = _ln_stats(x)
            xt = [with_ones(a) for a in split128(x)]
            lane_q = lax.broadcasted_iota(jnp.int32, (8, 128), 1)
            lo_half = lane_q < 64
            with scope('qproj'):
                KT = D // 128
                part = {}

                def q_tile(j, t0, t1, t2):
                    r1 = pltpu.roll(t1, 64, 1)
                    r2 = pltpu.roll(t2, 64, 1)
                    qbuf[2 * j, 0] = _u32(dup16(t0))
                    qbuf[2 * j, 1] = _u32(jnp.concatenate([jnp.where(lo_half, t1, 0.0), jnp.where(lo_half, 0.0, r1)], axis=0))
                    qbuf[2 * j + 1, 0] = _u32(dup16(jnp.where(lo_half, r1, r2)))
                    qbuf[2 * j + 1, 1] = _u32(jnp.concatenate([jnp.where(lo_half, r2, 0.0), jnp.where(lo_half, 0.0, t2)], axis=0))

                def q_pop(key, res):
                    n, k = key
                    part[n] = res if k == 0 else part[n] + res
                    if k == KT - 1:
                        part[n] = (part[n][0:8] - m_ * part[n][8:16]) * (rs_ * (SCALE * LOG2E))
                        j = n // 3
                        if all((3 * j + t) in part and done.get(3 * j + t) for t in range(3) if 3 * j + t != n):
                            q_tile(j, part[3 * j], part[3 * j + 1], part[3 * j + 2])
                        done[n] = True
                done = {}
                jobs = [[(xt[k], (lambda n=n, k=k: wq[k * 128:(k + 1) * 128, n * 128:(n + 1) * 128]), (n, k))
                         for n in range(m, 3 * H // 2, 4) for k in range(KT)] for m in range(4)]
                mxu_stream(jobs, q_pop)

            lane = lax.broadcasted_iota(jnp.int32, (1, 128), 1)
            grp = lane // 8
            diag = (lax.broadcasted_iota(jnp.int32, (8, 128), 0) == lax.broadcasted_iota(jnp.int32, (8, 128), 1) % 8)

            def u32(x):
                return _bf(x)

            def k_rhs(h, m, j):
                if j < 2:
                    return u32(k32[b * H + h, 2 * m + j, 0:64, :])
                return jnp.concatenate([u32(k32[b * H + h, 2 * m, 64:96, :]), u32(k32[b * H + h, 2 * m + 1, 64:96, :])], axis=0)

            def pop(m):
                return pltpu.matmul_pop_fifo((16, 128), F32, m)


            def st_kpop(h, kres):
                ss = []
                for m in range(4):
                    f0, f1, hf = kres[m]
                    ss.append(f0[0:8] + hf[0:8])
                    ss.append(f1[0:8] + hf[8:16])
                mx = ss[0]
                for c in range(NC):
                    sbuf[h & 1, :, c * 128:(c + 1) * 128] = ss[c]
                    if c:
                        mx = jnp.maximum(mx, ss[c])
                mbuf[h & 1] = mx

            def st_soft(h):
                mx = jnp.max(mbuf[h & 1], axis=-1, keepdims=True)
                ps = None
                for c in range(NC):
                    p = jnp.exp2(sbuf[h & 1, :, c * 128:(c + 1) * 128] - mx)
                    pbuf[h & 1, :, c * 128:(c + 1) * 128] = p
                    ps = p if ps is None else ps + p
                lbuf[h & 1] = ps

            def st_b1(h, lo=0, hi=DH // 16, do_l=True):
                p = pbuf[h & 1]
                if do_l:
                    l = jnp.sum(lbuf[h & 1], axis=-1, keepdims=True)
                    ilbuf[h & 3] = jnp.broadcast_to(1.0 / l, (8, 128))
                for r in range(lo, hi):
                    a0 = a1 = None
                    for c in range(NC):
                        w = v32[b * H + h, c, 8 * r:8 * r + 8, :]
                        pc = p[:, c * 128:(c + 1) * 128]
                        t0 = pltpu.unpack_elementwise(w, index=0, packed_dtype=BF, unpacked_dtype=F32) * pc
                        t1 = pltpu.unpack_elementwise(w, index=1, packed_dtype=BF, unpacked_dtype=F32) * pc
                        a0 = t0 if a0 is None else a0 + t0
                        a1 = t1 if a1 is None else a1 + t1
                    abuf[h & 1, 8 * r:8 * r + 8, :] = pltpu.pack_elementwise([a0, a1], packed_dtype=BF)

            def o_lhs(h, xres):
                il = ilbuf[h & 3]
                o0 = xres[0][0:8] * il
                o1 = xres[1][0:8] * il
                return [dup16(o0), jnp.concatenate([jnp.where(lo_half, o1, 0.0), jnp.where(lo_half, 0.0, o1)], axis=0).astype(BF)]

            WO_TILES = [(0,), (1,), (2,), (3,), (4,), (0, 1), (2, 3), (4, 4)]
            PROG = prog or [[('x', 0), ('k', 0), ('k', 1), ('k', 2), ('w', 0)],
                            [('x', 1), ('k', 0), ('k', 1), ('k', 2), ('w', 1)],
                            [('k', 0), ('k', 1), ('k', 2), ('w', 2), ('w', 3), ('w', 5)],
                            [('k', 0), ('k', 1), ('k', 2), ('w', 4), ('w', 6), ('w', 7)]]

            def wo_rhs(h, t):
                r0 = pl.multiple_of(h * (DH // 2), 32) if not isinstance(h, int) else h * (DH // 2)
                t = WO_TILES[t]
                if len(t) == 1:
                    return u32(wo32[t[0], pl.ds(r0, 64), :])
                return jnp.concatenate([u32(wo32[t[0], pl.ds(r0 + 64, 32), :]), u32(wo32[t[1], pl.ds(r0 + 64, 32), :])], axis=0)

            def step(i, acc, si=None):
                static = isinstance(i, int)
                if si is None and static:
                    si = i

                class Stage:
                    def __init__(self, d):
                        self.d = d
                live = lambda d: si is None or 0 <= si - d < H
                hk, hkp, hs_, hb, hx, hc, hcp = i, i - 1, i - 2, i - 3, i - 4, i - 5, i - 6
                ok = lambda h: live([d for d, v in enumerate((hk, hkp, hs_, hb, hx, hc, hcp)) if v is h][0])
                if ok(hk):
                    ql = [_bf(qbuf[hk, 0]), _bf(qbuf[hk, 1])]
                kres = [[None] * 3 for _ in range(4)]
                xres = [None, None]
                wres = [None] * 8
                ol = [None]

                def slot(m, kind, j):
                    if kind == 'k':
                        if ok(hkp) and not late_pop:
                            kres[m][j] = pop(m)
                        if ok(hk):
                            pltpu.matmul_push_rhs(k_rhs(hk, m, j), 0, m)
                            pltpu.matmul_lhs_fifo(ql[j // 2], m, load_staged_rhs=0)
                        if ok(hkp) and late_pop:
                            kres[m][j] = pop(m)
                    elif kind == 'x':
                        if ok(hc):
                            xres[j] = pop(m)
                        if ok(hx):
                            if j == 0:
                                a = _bf(abuf[hx & 1, 0:64, :])
                            else:
                                ah = _bf(abuf[hx & 1, 64:96, :])
                                a = jnp.concatenate([ah, ah], axis=0)
                            pltpu.matmul_push_rhs(a, 0, m, transpose=True)
                            pltpu.matmul_lhs_fifo(_bf(onesb[...]), m, load_staged_rhs=0)
                    else:
                        if ok(hcp) and not late_pop:
                            wres[j] = pop(m)
                        if ok(hc):
                            if ol[0] is None:
                                ol[0] = o_lhs(hc, xres)
                            pltpu.matmul_push_rhs(wo_rhs(hc, j), 0, m)
                            pltpu.matmul_lhs_fifo(ol[0][len(WO_TILES[j]) - 1], m, load_staged_rhs=0)
                        if ok(hcp) and late_pop:
                            wres[j] = pop(m)

                def part(t0, t1, g0, g1, tail):
                    for t in range(t0, t1):
                        for m in range(4):
                            if t < len(PROG[m]):
                                slot(m, *PROG[m][t])
                    if ok(hb): st_b1(hb, g0, g1, do_l=(g0 == 0))

                def fin(acc):
                    if ok(hcp):
                        outs = [None] * 5
                        for j, t in enumerate(WO_TILES):
                            r = wres[j]
                            pieces = [(t[0], r[0:8])] if (len(t) == 1 or t[0] == t[1]) else [(t[0], r[0:8]), (t[1], r[8:16])]
                            for n, v in pieces:
                                outs[n] = v if outs[n] is None else outs[n] + v
                        if acc_mem:
                            accb[...] = accb[...] + jnp.concatenate(outs, axis=1)
                        else:
                            acc = acc + jnp.concatenate(outs, axis=1)
                    return acc

                if split and not static:
                    bounds = split
                    prev_t, prev_g = 0, 0
                    for idx, (t1, g1) in enumerate(bounds):
                        if idx == 0:
                            part(prev_t, t1, prev_g, g1, False)
                            if ok(hs_): st_soft(hs_)
                        else:
                            def blk(_, c, a=prev_t, t1=t1, g0=prev_g, g1=g1, last=(idx == len(bounds) - 1)):
                                part(a, t1, g0, g1, last)
                                if last:
                                    fin(0)
                                    if ok(hkp): st_kpop(hkp, kres)
                                return c
                            lax.fori_loop(0, jnp.minimum(b + 1, 1), blk, 0)
                        prev_t, prev_g = t1, g1
                    return acc
                def mx():
                    if slot_major:
                        for t in range(6):
                            for m in morder:
                                if t < len(PROG[m]):
                                    slot(m, *PROG[m][t])
                    else:
                        tm = [0] * 4
                        pos = [0] * 4
                        while any(pos[m] < len(PROG[m]) for m in range(4)):
                            cand = [m for m in morder if pos[m] < len(PROG[m])]
                            m = min(cand, key=lambda q: tm[q])
                            slot(m, *PROG[m][pos[m]])
                            tm[m] += 2 if PROG[m][pos[m]][0] == 'x' else 1
                            pos[m] += 1
                for what in order:
                    if what == 'm': mx()
                    elif what == 'b' and ok(hb): st_b1(hb)
                    elif what == 'f': acc = fin(acc)
                    elif what == 's' and ok(hs_): st_soft(hs_)
                    elif what == 'k' and ok(hkp): st_kpop(hkp, kres)
                return acc

            def vwait(h0):
                groups = {}
                for bb in range(B):
                    for (hh, n) in VCH[bb]:
                        if hh == h0:
                            groups.setdefault(n, []).append(bb)
                for n, bs in groups.items():
                    cond = first
                    if len(bs) < B:
                        c = None
                        for bb in bs:
                            c = (b == bb) if c is None else jnp.logical_or(c, b == bb)
                        cond = jnp.logical_and(first, c)
                    @pl.when(cond)
                    def _():
                        kvall(vbuf, sem_v, b, h0, n).wait()

            if acc_mem:
                accb[...] = jnp.zeros((8, D), F32)
                acc = 0
            else:
                acc = jnp.zeros((8, D), F32)
            vstarts = sorted({h0 for bb in range(B) for (h0, n) in VCH[bb]})
            with scope('attn'):
                i = 0
                while i < H + 6:
                    if (i - 3) in vstarts:
                        vwait(i - 3)
                    nxt = min([h0 + 3 for h0 in vstarts if h0 + 3 > i] + [H])
                    if 6 <= i < H and nxt - i >= 2 * unroll:
                        cnt = (nxt - i) // unroll
                        def multi(j, acc, i0=i):
                            for u in range(unroll):
                                acc = step(i0 + j * unroll + u, acc)
                            return acc
                        acc = lax.fori_loop(0, cnt, multi, acc)
                        i += cnt * unroll
                    else:
                        if isolate and i >= iso_from:
                            acc = lax.fori_loop(i, i + jnp.minimum(b + 1, 1), lambda ii, a, i=i: step(ii, a, si=i), acc)
                        else:
                            acc = step(i, acc)
                        i += 1
            with scope('ffn'):
                x = x + (accb[...] if acc_mem else acc)
                m2, rs2 = _ln_stats(x)
                xn32 = ((x - m2) * rs2).astype(BF).astype(F32)
                r = jnp.sum(xn32 * wr32, axis=-1, keepdims=True)
                xt = [with_ones(a) for a in split128(x)]
                KT, NF, NO = D // 128, F // 128, D // 128
                gu = {}
                hs = {}
                ys = {}

                def f_pop(key, res):
                    kind, n, k = key
                    v = res[0:8]
                    if kind < 2:
                        gu[kind, n] = res if k == 0 else gu[kind, n] + res
                        if k == KT - 1:
                            gu[kind, n] = (gu[kind, n][0:8] - m2 * gu[kind, n][8:16]) * rs2
                        if kind == 1 and k == KT - 1:
                            gt, up = gu[0, n], gu[1, n]
                            hs[n] = dup16(gt * jax.nn.sigmoid(gt) * up)
                    else:
                        ys[n] = v if n not in ys else ys[n] + v
                jobs = []
                for m in range(4):
                    jm = []
                    for n in range(m, NF, 4):
                        for kind, w in ((0, wg), (1, wu)):
                            for k in range(KT):
                                jm.append((xt[k], (lambda w=w, n=n, k=k: w[k * 128:(k + 1) * 128, n * 128:(n + 1) * 128]), (kind, n, k)))
                    for k in range(m, NF, 4):
                        for n in range(NO):
                            jm.append(((lambda k=k: hs[k]), (lambda n=n, k=k: wd[k * 128:(k + 1) * 128, n * 128:(n + 1) * 128]), (2, n, k)))
                    jobs.append(jm)
                mxu_stream(jobs, f_pop)
                y = jnp.concatenate([ys[n] for n in range(NO)], axis=1)
                y = y * jax.nn.sigmoid(r)
                x = x + (xn32 + (xn32 * 0.0 + y))
                xs[pl.ds(b, 1), :] = x[0:1, :]
            return carry

        def layer(it, carry):
            with scope('layer'):
                return layer_(it, carry)

        lax.fori_loop(0, 2 * B, layer, 0)
        out_ref[...] = xs[0:4, :].astype(BF)

    @jax.jit
    def kernel_fn(A_x, A_k_cache, A_v_cache, A_wq, A_wo, B_x, B_w_r, B_w_gate, B_w_up, B_w_down):
        kt = jnp.swapaxes(A_k_cache, 2, 3)
        vt = jnp.swapaxes(A_v_cache, 2, 3)
        x2 = A_x.reshape(B, D)
        anyspec = pl.BlockSpec(memory_space=pl.ANY)
        out = pl.pallas_call(
            _kernel,
            out_shape=jax.ShapeDtypeStruct((B, D), BF), grid=(1,),
            in_specs=[anyspec] * 9,
            out_specs=pl.BlockSpec(memory_space=pltpu.VMEM),
            scratch_shapes=[
                pltpu.VMEM((B, D), BF),
                pltpu.VMEM((B * H, NC, DH, 128), BF),
                pltpu.VMEM((B * H, NC, DH, 128), BF),
                pltpu.VMEM((D, H * DH), BF),
                pltpu.VMEM((H * DH, D), BF),
                pltpu.VMEM((D // 128, H * DH, 128), BF),
                pltpu.VMEM((D,), BF),
                pltpu.VMEM((D, F), BF),
                pltpu.VMEM((D, F), BF),
                pltpu.VMEM((F, D), BF),
                pltpu.VMEM((8, D), F32),
                pltpu.VMEM((8, D), F32),
                pltpu.VMEM((8, 128), jnp.uint32),
                pltpu.VMEM((H, 2, 8, 128), jnp.uint32),
                pltpu.VMEM((4, 8, 128), F32),
                pltpu.VMEM((2, 8, W), F32),
                pltpu.VMEM((2, 8, 128), F32),
                pltpu.VMEM((2, 8, W), F32),
                pltpu.VMEM((2, 8, 128), F32),
                pltpu.VMEM((2, DH // 2, 128), jnp.uint32),
                pltpu.SemaphoreType.DMA((7,)),
                pltpu.SemaphoreType.DMA((len(KIDX),)),
                pltpu.SemaphoreType.DMA((len(VIDX),)),
            ],
            compiler_params=pltpu.CompilerParams(vmem_limit_bytes=127 * 1024 * 1024),
        )(x2, kt, vt, A_wq, A_wo, B_w_r, B_w_gate, B_w_up, B_w_down)
        return out.reshape(B, 1, D)
    return kernel_fn


_impl = make_kernel()


@jax.jit
def pallas_interleave_layers__sliding_block_cached__moe_arch_mod__decode_kernel(
    A_x, A_k_cache, A_v_cache, A_wq, A_wo, B_x, B_w_r, B_w_gate, B_w_up, B_w_down
):
    return _impl(A_x, A_k_cache, A_v_cache, A_wq, A_wo, B_x, B_w_r, B_w_gate, B_w_up, B_w_down)
```

```python
import functools

import jax
import jax.numpy as jnp
from jax import lax
import jax.experimental.pallas as pl
import jax.experimental.pallas.tpu as pltpu

B, D, H, DH, SK, W, F = 4, 640, 32, 192, 4096, 1024, 1536
NC = W // 128
NMXU = 4
SCALE = DH ** -0.5
LOG2E = 1.4426950408889634
EPS = 1e-5
BF = jnp.bfloat16
F32 = jnp.float32

V_LAST = ((0, 16), (16, 8), (24, 4), (28, 2), (30, 1), (31, 1))
V_LAST_ISSUE = 2 * (B - 2)
SEM_W = 0
SEM_K = tuple(1 + b for b in range(B))
SEM_V = tuple(1 + B + b for b in range(B - 1))
SEM_V_LAST = (SEM_V[0], SEM_V[1], SEM_K[0], SEM_K[1], SEM_W, 2 * B)
NSEM = 2 * B + 1

WO_TILES = ((0,), (1,), (2,), (3,), (4,), (0, 1), (2, 3), (4, 4))
MXU_PROGRAM = (
    (("x", 0), ("k", 0), ("k", 1), ("k", 2), ("w", 0)),
    (("x", 1), ("k", 0), ("k", 1), ("k", 2), ("w", 1)),
    (("k", 0), ("k", 1), ("k", 2), ("w", 2), ("w", 3), ("w", 5)),
    (("k", 0), ("k", 1), ("k", 2), ("w", 4), ("w", 6), ("w", 7)),
)
DEPTH = 6
V_STAGE = 3
PEEL_FROM = 30
POP_LAG = 4


def _ln_stats(x):
    t = [x[:, i:i + 128] for i in range(0, x.shape[1], 128)]
    s1 = functools.reduce(jnp.add, t)
    s2 = functools.reduce(jnp.add, [a * a for a in t])
    n = x.shape[1]
    m = jnp.sum(s1, axis=-1, keepdims=True) * (1.0 / n)
    q = jnp.sum(s2, axis=-1, keepdims=True) * (1.0 / n)
    v = jnp.maximum(q - m * m, 0.0)
    return m, lax.rsqrt(v + EPS)


def _bf(u):
    return pltpu.bitcast(u, BF)


def _u32(x):
    return pltpu.bitcast(x.astype(BF), jnp.uint32)


def _tiles(a):
    return [a[:, i:i + 128] for i in range(0, a.shape[1], 128)]


def _dup16(a):
    return jnp.concatenate([a, a], axis=0).astype(BF)


def _with_ones(a):
    return jnp.concatenate([a, jnp.ones_like(a)], axis=0).astype(BF)


def _mxu_stream(jobs, on_result):
    for t in range(max(len(j) for j in jobs) + POP_LAG):
        for m in range(NMXU):
            if 0 <= t - POP_LAG < len(jobs[m]):
                on_result(jobs[m][t - POP_LAG][2], pltpu.matmul_pop_fifo((16, 128), F32, m))
            if t < len(jobs[m]):
                lhs, rhs, _ = jobs[m][t]
                pltpu.matmul_push_rhs(rhs(), 0, m)
                pltpu.matmul_lhs_fifo(lhs() if callable(lhs) else lhs, m, load_staged_rhs=0)


def _kernel(x_hbm, k_hbm, v_hbm, wq_hbm, wo_hbm, wr_hbm, wg_hbm, wu_hbm, wd_hbm,
            out_ref,
            xb, kbuf, vbuf, wq, wo_nat, wo, wr, wg, wu, wd,
            xs, accb, onesb, qbuf, ilbuf, sbuf, mbuf, pbuf, lbuf, abuf, sems):
    weights = [pltpu.make_async_copy(s, d, sems.at[SEM_W]) for s, d in (
        (x_hbm, xb), (wr_hbm, wr), (wq_hbm, wq), (wo_hbm, wo_nat), (wg_hbm, wg), (wu_hbm, wu), (wd_hbm, wd))]

    def start_kv(hbm, buf, sem, b, h0, n):
        def tile(c, carry):
            pltpu.make_async_copy(
                hbm.at[b, pl.ds(h0, n), :, pl.ds(pl.multiple_of(SK - W + c * 128, 128), 128)],
                buf.at[pl.ds(b * H + h0, n), c], sems.at[sem]).start()
            return carry
        lax.fori_loop(0, NC, tile, 0)

    def wait_kv(buf, sem, b, h0, n):
        whole = buf.at[pl.ds(b * H + h0, n)]
        pltpu.make_async_copy(whole, whole, sems.at[sem]).wait()

    for c in weights:
        c.start()
    for b in range(B):
        start_kv(k_hbm, kbuf, SEM_K[b], b, 0, H)
        if b < B - 1:
            start_kv(v_hbm, vbuf, SEM_V[b], b, 0, H)
    for c in weights:
        c.wait()

    xs[...] = jnp.zeros((8, D), F32)
    xs[0:B, :] = xb[...].astype(F32)
    wr32 = jnp.broadcast_to(wr[...].astype(F32).reshape(1, D), (8, D))
    onesb[...] = pltpu.bitcast(jnp.ones((16, 128), BF), jnp.uint32)

    def retile(i, carry):
        r0 = pl.multiple_of(i * 256, 256)
        for n in range(D // 128):
            wo[n, pl.ds(r0, 256), :] = wo_nat[pl.ds(r0, 256), n * 128:(n + 1) * 128]
        return carry
    lax.fori_loop(0, H * DH // 256, retile, 0)

    sbuf, mbuf, pbuf, lbuf, abuf, ilbuf = [
        pltpu.annotate(r, no_hazard=True) for r in (sbuf, mbuf, pbuf, lbuf, abuf, ilbuf)]
    k32 = kbuf.bitcast(jnp.uint32)
    v32 = vbuf.bitcast(jnp.uint32)
    wo32 = wo.bitcast(jnp.uint32)

    def layer(it, carry):
        b = it // 2
        first = (it % 2) == 0

        @pl.when(it == V_LAST_ISSUE)
        def _():
            for (h0, n), sem in zip(V_LAST, SEM_V_LAST):
                start_kv(v_hbm, vbuf, sem, B - 1, h0, n)

        @pl.when(first)
        def _():
            wait_kv(kbuf, 1 + b, b, 0, H)

        x = jnp.broadcast_to(xs[pl.ds(b, 1), :], (8, D))
        lo_half = lax.broadcasted_iota(jnp.int32, (8, 128), 1) < 64
        KT = D // 128

        mean, rstd = _ln_stats(x)
        xt = [_with_ones(a) for a in _tiles(x)]
        part, done = {}, set()

        def q_pair(j, t0, t1, t2):
            r1 = pltpu.roll(t1, 64, 1)
            r2 = pltpu.roll(t2, 64, 1)
            qbuf[2 * j, 0] = _u32(_dup16(t0))
            qbuf[2 * j, 1] = _u32(jnp.concatenate([jnp.where(lo_half, t1, 0.0), jnp.where(lo_half, 0.0, r1)], axis=0))
            qbuf[2 * j + 1, 0] = _u32(_dup16(jnp.where(lo_half, r1, r2)))
            qbuf[2 * j + 1, 1] = _u32(jnp.concatenate([jnp.where(lo_half, r2, 0.0), jnp.where(lo_half, 0.0, t2)], axis=0))

        def q_result(key, res):
            n, k = key
            part[n] = res if k == 0 else part[n] + res
            if k == KT - 1:
                part[n] = (part[n][0:8] - mean * part[n][8:16]) * (rstd * (SCALE * LOG2E))
                done.add(n)
                j = n // 3
                if all(3 * j + t in done for t in range(3)):
                    q_pair(j, part[3 * j], part[3 * j + 1], part[3 * j + 2])

        _mxu_stream([[(xt[k], (lambda n=n, k=k: wq[k * 128:(k + 1) * 128, n * 128:(n + 1) * 128]), (n, k))
                      for n in range(m, H * DH // 128, NMXU) for k in range(KT)] for m in range(NMXU)], q_result)

        def k_rhs(h, m, j):
            if j < 2:
                return _bf(k32[b * H + h, 2 * m + j, 0:64, :])
            return jnp.concatenate([_bf(k32[b * H + h, 2 * m, 64:96, :]), _bf(k32[b * H + h, 2 * m + 1, 64:96, :])], axis=0)

        def wo_rhs(h, j):
            r0 = h * (DH // 2)
            if not isinstance(h, int):
                r0 = pl.multiple_of(r0, 32)
            t = WO_TILES[j]
            if len(t) == 1:
                return _bf(wo32[t[0], pl.ds(r0, 64), :])
            return jnp.concatenate([_bf(wo32[t[0], pl.ds(r0 + 64, 32), :]), _bf(wo32[t[1], pl.ds(r0 + 64, 32), :])], axis=0)

        def scores(h, kres):
            ss = []
            for m in range(NMXU):
                f0, f1, hf = kres[m]
                ss += [f0[0:8] + hf[0:8], f1[0:8] + hf[8:16]]
            mx = ss[0]
            for c in range(NC):
                sbuf[h & 1, :, c * 128:(c + 1) * 128] = ss[c]
                if c:
                    mx = jnp.maximum(mx, ss[c])
            mbuf[h & 1] = mx

        def softmax(h):
            mx = jnp.max(mbuf[h & 1], axis=-1, keepdims=True)
            ps = None
            for c in range(NC):
                p = jnp.exp2(sbuf[h & 1, :, c * 128:(c + 1) * 128] - mx)
                pbuf[h & 1, :, c * 128:(c + 1) * 128] = p
                ps = p if ps is None else ps + p
            lbuf[h & 1] = ps

        def p_times_v(h):
            p = pbuf[h & 1]
            l = jnp.sum(lbuf[h & 1], axis=-1, keepdims=True)
            ilbuf[h & 3] = jnp.broadcast_to(1.0 / l, (8, 128))
            for r in range(DH // 16):
                a0 = a1 = None
                for c in range(NC):
                    w = v32[b * H + h, c, 8 * r:8 * r + 8, :]
                    pc = p[:, c * 128:(c + 1) * 128]
                    t0 = pltpu.unpack_elementwise(w, index=0, packed_dtype=BF, unpacked_dtype=F32) * pc
                    t1 = pltpu.unpack_elementwise(w, index=1, packed_dtype=BF, unpacked_dtype=F32) * pc
                    a0 = t0 if a0 is None else a0 + t0
                    a1 = t1 if a1 is None else a1 + t1
                abuf[h & 1, 8 * r:8 * r + 8, :] = pltpu.pack_elementwise([a0, a1], packed_dtype=BF)

        def o_lhs(h, xres):
            il = ilbuf[h & 3]
            o0 = xres[0][0:8] * il
            o1 = xres[1][0:8] * il
            return [_dup16(o0),
                    jnp.concatenate([jnp.where(lo_half, o1, 0.0), jnp.where(lo_half, 0.0, o1)], axis=0).astype(BF)]

        def step(i, carry, at=None):
            live = [at is None or 0 <= at - d < H for d in range(DEPTH + 1)]
            h_k, h_s, h_p, h_v, h_x, h_o, h_a = (i - d for d in range(DEPTH + 1))
            if live[0]:
                ql = [_bf(qbuf[h_k, 0]), _bf(qbuf[h_k, 1])]
            kres = [[None] * 3 for _ in range(NMXU)]
            xres = [None, None]
            wres = [None] * len(WO_TILES)
            ol = []

            def slot(m, kind, j):
                if kind == "k":
                    if live[0]:
                        pltpu.matmul_push_rhs(k_rhs(h_k, m, j), 0, m)
                        pltpu.matmul_lhs_fifo(ql[j // 2], m, load_staged_rhs=0)
                    if live[1]:
                        kres[m][j] = pltpu.matmul_pop_fifo((16, 128), F32, m)
                elif kind == "x":
                    if live[5]:
                        xres[j] = pltpu.matmul_pop_fifo((16, 128), F32, m)
                    if live[4]:
                        if j == 0:
                            a = _bf(abuf[h_x & 1, 0:64, :])
                        else:
                            ah = _bf(abuf[h_x & 1, 64:96, :])
                            a = jnp.concatenate([ah, ah], axis=0)
                        pltpu.matmul_push_rhs(a, 0, m, transpose=True)
                        pltpu.matmul_lhs_fifo(_bf(onesb[...]), m, load_staged_rhs=0)
                else:
                    if live[5]:
                        if not ol:
                            ol.extend(o_lhs(h_o, xres))
                        pltpu.matmul_push_rhs(wo_rhs(h_o, j), 0, m)
                        pltpu.matmul_lhs_fifo(ol[len(WO_TILES[j]) - 1], m, load_staged_rhs=0)
                    if live[6]:
                        wres[j] = pltpu.matmul_pop_fifo((16, 128), F32, m)

            for t in range(6):
                for m in range(NMXU):
                    if t < len(MXU_PROGRAM[m]):
                        slot(m, *MXU_PROGRAM[m][t])
            if live[6]:
                outs = [None] * (D // 128)
                for t, r in zip(WO_TILES, wres):
                    pieces = [(t[0], r[0:8])] if (len(t) == 1 or t[0] == t[1]) else [(t[0], r[0:8]), (t[1], r[8:16])]
                    for n, v in pieces:
                        outs[n] = v if outs[n] is None else outs[n] + v
                accb[...] = accb[...] + jnp.concatenate(outs, axis=1)
            if live[3]:
                p_times_v(h_v)
            if live[2]:
                softmax(h_p)
            if live[1]:
                scores(h_s, kres)
            return carry

        def wait_v(h0):
            if h0 == 0:
                @pl.when(jnp.logical_and(first, b < B - 1))
                def _():
                    wait_kv(vbuf, 1 + B + b, b, 0, H)
            for (hh, n), sem in zip(V_LAST, SEM_V_LAST):
                if hh == h0:
                    @pl.when(jnp.logical_and(first, b == B - 1))
                    def _():
                        wait_kv(vbuf, sem, b, hh, n)

        accb[...] = jnp.zeros((8, D), F32)
        v_starts = [h0 for h0, _ in V_LAST]
        once = jnp.minimum(b + 1, 1)
        i = 0
        while i < H + DEPTH:
            if i - V_STAGE in v_starts:
                wait_v(i - V_STAGE)
            nxt = min([h0 + V_STAGE for h0 in v_starts if h0 + V_STAGE > i] + [H])
            if DEPTH <= i < H and nxt - i >= 2:
                lax.fori_loop(i, nxt, step, 0)
                i = nxt
            else:
                if i >= PEEL_FROM:
                    lax.fori_loop(i, i + once, functools.partial(step, at=i), 0)
                else:
                    step(i, 0, at=i)
                i += 1

        x = x + accb[...]
        mean, rstd = _ln_stats(x)
        xn = ((x - mean) * rstd).astype(BF).astype(F32)
        r = jnp.sum(xn * wr32, axis=-1, keepdims=True)
        xt = [_with_ones(a) for a in _tiles(x)]
        NF, NO = F // 128, D // 128
        gu, hs, ys = {}, {}, {}

        def f_result(key, res):
            kind, n, k = key
            if kind < 2:
                gu[kind, n] = res if k == 0 else gu[kind, n] + res
                if k == KT - 1:
                    gu[kind, n] = (gu[kind, n][0:8] - mean * gu[kind, n][8:16]) * rstd
                    if kind == 1:
                        g, u = gu[0, n], gu[1, n]
                        hs[n] = _dup16(g * jax.nn.sigmoid(g) * u)
            else:
                ys[n] = res[0:8] if n not in ys else ys[n] + res[0:8]

        jobs = []
        for m in range(NMXU):
            jm = []
            for n in range(m, NF, NMXU):
                for kind, w in ((0, wg), (1, wu)):
                    for k in range(KT):
                        jm.append((xt[k], (lambda w=w, n=n, k=k: w[k * 128:(k + 1) * 128, n * 128:(n + 1) * 128]), (kind, n, k)))
            for k in range(m, NF, NMXU):
                for n in range(NO):
                    jm.append(((lambda k=k: hs[k]), (lambda n=n, k=k: wd[k * 128:(k + 1) * 128, n * 128:(n + 1) * 128]), (2, n, k)))
            jobs.append(jm)
        _mxu_stream(jobs, f_result)
        y = jnp.concatenate([ys[n] for n in range(NO)], axis=1) * jax.nn.sigmoid(r)
        x = x + (xn + (xn * 0.0 + y))
        xs[pl.ds(b, 1), :] = x[0:1, :]
        return carry

    lax.fori_loop(0, 2 * B, layer, 0)
    out_ref[...] = xs[0:B, :].astype(BF)


@jax.jit
def pallas_interleave_layers__sliding_block_cached__moe_arch_mod__decode_kernel(
    A_x, A_k_cache, A_v_cache, A_wq, A_wo, B_x, B_w_r, B_w_gate, B_w_up, B_w_down
):
    del B_x
    kt = jnp.swapaxes(A_k_cache, 2, 3)
    vt = jnp.swapaxes(A_v_cache, 2, 3)
    anyspec = pl.BlockSpec(memory_space=pl.ANY)
    out = pl.pallas_call(
        _kernel,
        out_shape=jax.ShapeDtypeStruct((B, D), BF),
        grid=(1,),
        in_specs=[anyspec] * 9,
        out_specs=pl.BlockSpec(memory_space=pltpu.VMEM),
        scratch_shapes=[
            pltpu.VMEM((B, D), BF),
            pltpu.VMEM((B * H, NC, DH, 128), BF),
            pltpu.VMEM((B * H, NC, DH, 128), BF),
            pltpu.VMEM((D, H * DH), BF),
            pltpu.VMEM((H * DH, D), BF),
            pltpu.VMEM((D // 128, H * DH, 128), BF),
            pltpu.VMEM((D,), BF),
            pltpu.VMEM((D, F), BF),
            pltpu.VMEM((D, F), BF),
            pltpu.VMEM((F, D), BF),
            pltpu.VMEM((8, D), F32),
            pltpu.VMEM((8, D), F32),
            pltpu.VMEM((8, 128), jnp.uint32),
            pltpu.VMEM((H, 2, 8, 128), jnp.uint32),
            pltpu.VMEM((4, 8, 128), F32),
            pltpu.VMEM((2, 8, W), F32),
            pltpu.VMEM((2, 8, 128), F32),
            pltpu.VMEM((2, 8, W), F32),
            pltpu.VMEM((2, 8, 128), F32),
            pltpu.VMEM((2, DH // 2, 128), jnp.uint32),
            pltpu.SemaphoreType.DMA((NSEM,)),
        ],
        compiler_params=pltpu.CompilerParams(vmem_limit_bytes=127 * 1024 * 1024),
    )(A_x.reshape(B, D), kt, vt, A_wq, A_wo, B_w_r, B_w_gate, B_w_up, B_w_down)
    return out.reshape(B, 1, D)
```

```python
import functools

import jax
import jax.numpy as jnp
from jax import lax
import jax.experimental.pallas as pl
import jax.experimental.pallas.tpu as pltpu

B, D, H, DH, SK, W, F = 4, 640, 32, 192, 4096, 1024, 1536
NC = W // 128
SCALE = DH ** -0.5
LOG2E = 1.4426950408889634
EPS = 1e-5
BF = jnp.bfloat16
F32 = jnp.float32

V_LAST = ((0, 16), (16, 8), (24, 4), (28, 2), (30, 1), (31, 1))
V_LAST_ISSUE = 2 * (B - 2)
SEM_W = 0
SEM_K = tuple(1 + b for b in range(B))
SEM_V = tuple(1 + B + b for b in range(B - 1))
SEM_V_LAST = (SEM_V[0], SEM_V[1], SEM_K[0], SEM_K[1], SEM_W, 2 * B)
NSEM = 2 * B + 1

WO_TILES = ((0,), (1,), (2,), (3,), (4,), (0, 1), (2, 3), (4, 4))
G = 2
NG = H // G
DEPTH = 4
V_STAGE = 2


def _ln_stats(x):
    t = [x[:, i:i + 128] for i in range(0, x.shape[1], 128)]
    s1 = functools.reduce(jnp.add, t)
    s2 = functools.reduce(jnp.add, [a * a for a in t])
    n = x.shape[1]
    m = jnp.sum(s1, axis=-1, keepdims=True) * (1.0 / n)
    q = jnp.sum(s2, axis=-1, keepdims=True) * (1.0 / n)
    v = jnp.maximum(q - m * m, 0.0)
    return m, lax.rsqrt(v + EPS)


def _bf(u):
    return pltpu.bitcast(u, BF)


def _u32(x):
    return pltpu.bitcast(x.astype(BF), jnp.uint32)


def _tiles(a):
    return [a[:, i:i + 128] for i in range(0, a.shape[1], 128)]


def _dup16(a):
    return jnp.concatenate([a, a], axis=0).astype(BF)


def _with_ones(a):
    return jnp.concatenate([a, jnp.ones_like(a)], axis=0).astype(BF)


def _dot(a, b):
    return jnp.dot(a, b, preferred_element_type=F32)


def _kernel(x_hbm, k_hbm, v_hbm, wq_hbm, wo_hbm, wr_hbm, wg_hbm, wu_hbm, wd_hbm,
            out_ref,
            xb, kbuf, vbuf, wq, wo_nat, wo, wr, wg, wu, wd,
            xs, accb, onesb, qbuf, ilbuf, sbuf, mbuf, pbuf, lbuf, abuf, obuf, sems):
    weights = [pltpu.make_async_copy(s, d, sems.at[SEM_W]) for s, d in (
        (x_hbm, xb), (wr_hbm, wr), (wq_hbm, wq), (wo_hbm, wo_nat), (wg_hbm, wg), (wu_hbm, wu), (wd_hbm, wd))]

    def start_kv(hbm, buf, sem, b, h0, n):
        def tile(c, carry):
            pltpu.make_async_copy(
                hbm.at[b, pl.ds(h0, n), :, pl.ds(pl.multiple_of(SK - W + c * 128, 128), 128)],
                buf.at[pl.ds(b * H + h0, n), c], sems.at[sem]).start()
            return carry
        lax.fori_loop(0, NC, tile, 0)

    def wait_kv(buf, sem, b, h0, n):
        whole = buf.at[pl.ds(b * H + h0, n)]
        pltpu.make_async_copy(whole, whole, sems.at[sem]).wait()

    for c in weights:
        c.start()
    for b in range(B):
        start_kv(k_hbm, kbuf, SEM_K[b], b, 0, H)
        if b < B - 1:
            start_kv(v_hbm, vbuf, SEM_V[b], b, 0, H)
    for c in weights:
        c.wait()

    xs[...] = jnp.zeros((8, D), F32)
    xs[0:B, :] = xb[...].astype(F32)
    wr32 = jnp.broadcast_to(wr[...].astype(F32).reshape(1, D), (8, D))
    onesb[...] = pltpu.bitcast(jnp.ones((16, 128), BF), jnp.uint32)

    def retile(i, carry):
        r0 = pl.multiple_of(i * 256, 256)
        for n in range(D // 128):
            wo[n, pl.ds(r0, 256), :] = wo_nat[pl.ds(r0, 256), n * 128:(n + 1) * 128]
        return carry
    lax.fori_loop(0, H * DH // 256, retile, 0)

    k32 = kbuf.bitcast(jnp.uint32)
    v32 = vbuf.bitcast(jnp.uint32)
    wo32 = wo.bitcast(jnp.uint32)

    def layer(it, carry):
        b = it // 2
        first = (it % 2) == 0

        @pl.when(it == V_LAST_ISSUE)
        def _():
            for (h0, n), sem in zip(V_LAST, SEM_V_LAST):
                start_kv(v_hbm, vbuf, sem, B - 1, h0, n)

        @pl.when(first)
        def _():
            wait_kv(kbuf, 1 + b, b, 0, H)

        x = jnp.broadcast_to(xs[pl.ds(b, 1), :], (8, D))
        lo_half = lax.broadcasted_iota(jnp.int32, (8, 128), 1) < 64
        KT = D // 128

        mean, rstd = _ln_stats(x)
        xt = [_with_ones(a) for a in _tiles(x)]
        part, done = {}, set()

        def q_pair(j, t0, t1, t2):
            r1 = pltpu.roll(t1, 64, 1)
            r2 = pltpu.roll(t2, 64, 1)
            qbuf[2 * j, 0] = _u32(_dup16(t0))
            qbuf[2 * j, 1] = _u32(jnp.concatenate([jnp.where(lo_half, t1, 0.0), jnp.where(lo_half, 0.0, r1)], axis=0))
            qbuf[2 * j + 1, 0] = _u32(_dup16(jnp.where(lo_half, r1, r2)))
            qbuf[2 * j + 1, 1] = _u32(jnp.concatenate([jnp.where(lo_half, r2, 0.0), jnp.where(lo_half, 0.0, t2)], axis=0))

        def q_result(key, res):
            n, k = key
            part[n] = res if k == 0 else part[n] + res
            if k == KT - 1:
                part[n] = (part[n][0:8] - mean * part[n][8:16]) * (rstd * (SCALE * LOG2E))
                done.add(n)
                j = n // 3
                if all(3 * j + t in done for t in range(3)):
                    q_pair(j, part[3 * j], part[3 * j + 1], part[3 * j + 2])

        for n in range(H * DH // 128):
            for k in range(KT):
                q_result((n, k), _dot(xt[k], wq[k * 128:(k + 1) * 128, n * 128:(n + 1) * 128]))

        def k_rhs(h, m, j):
            if j < 2:
                return _bf(k32[b * H + h, 2 * m + j, 0:64, :])
            return jnp.concatenate([_bf(k32[b * H + h, 2 * m, 64:96, :]), _bf(k32[b * H + h, 2 * m + 1, 64:96, :])], axis=0)

        def wo_rhs(h, j):
            r0 = h * (DH // 2)
            if not isinstance(h, int):
                r0 = pl.multiple_of(r0, 32)
            t = WO_TILES[j]
            if len(t) == 1:
                return _bf(wo32[t[0], pl.ds(r0, 64), :])
            return jnp.concatenate([_bf(wo32[t[0], pl.ds(r0 + 64, 32), :]), _bf(wo32[t[1], pl.ds(r0 + 64, 32), :])], axis=0)

        def scores(h, sl):
            ql = [_bf(qbuf[h, 0]), _bf(qbuf[h, 1])]
            mx = None
            for m in range(NC // 2):
                hf = _dot(ql[1], k_rhs(h, m, 2))
                for j in range(2):
                    sc = _dot(ql[0], k_rhs(h, m, j))[0:8] + hf[8 * j:8 * j + 8]
                    c = 2 * m + j
                    sbuf[sl, :, c * 128:(c + 1) * 128] = sc
                    mx = sc if mx is None else jnp.maximum(mx, sc)
            mbuf[sl] = mx

        def softmax(sl):
            mx = jnp.max(mbuf[sl], axis=-1, keepdims=True)
            ps = None
            for c in range(NC):
                p = jnp.exp2(sbuf[sl, :, c * 128:(c + 1) * 128] - mx)
                pbuf[sl, :, c * 128:(c + 1) * 128] = p
                ps = p if ps is None else ps + p
            lbuf[sl] = ps

        def p_times_v(h, sl):
            p = pbuf[sl]
            l = jnp.sum(lbuf[sl], axis=-1, keepdims=True)
            ilbuf[sl] = jnp.broadcast_to(1.0 / l, (8, 128))
            for r in range(DH // 16):
                a = None
                for c in range(NC):
                    t = vbuf[b * H + h, c, 16 * r:16 * r + 16, :].astype(F32).reshape(2, 8, 128) * p[None, :, c * 128:(c + 1) * 128]
                    a = t if a is None else a + t
                abuf[sl, 16 * r:16 * r + 16, :] = a.reshape(16, 128)

        lane = lax.broadcasted_iota(jnp.int32, (8, 128), 1)
        grp = lane // 8
        diag = lax.broadcasted_iota(jnp.int32, (8, 128), 0) == lane % 8

        def head_out(sl):
            d0 = d1 = jnp.zeros((8, 128), F32)
            for g in range(DH // 8):
                red = jnp.sum(abuf[sl, 8 * g:8 * g + 8, :], axis=-1, keepdims=True)
                if g < 16:
                    d0 = jnp.where(grp == g, red, d0)
                else:
                    d1 = jnp.where(grp % 8 == g - 16, red, d1)
            il = ilbuf[sl]
            o1 = d1 * il
            obuf[sl, 0] = _u32(_dup16(jnp.where(diag, d0 * il, 0.0)))
            obuf[sl, 1] = _u32(jnp.concatenate([jnp.where(diag & lo_half, o1, 0.0), jnp.where(diag & ~lo_half, o1, 0.0)], axis=0))

        def project(h, sl):
            ol = [_bf(obuf[sl, 0]), _bf(obuf[sl, 1])]
            outs = [None] * (D // 128)
            for j, t in enumerate(WO_TILES):
                r = _dot(ol[len(t) - 1], wo_rhs(h, j))
                pieces = [(t[0], r[0:8])] if (len(t) == 1 or t[0] == t[1]) else [(t[0], r[0:8]), (t[1], r[8:16])]
                for n, v in pieces:
                    outs[n] = v if outs[n] is None else outs[n] + v
            return jnp.concatenate(outs, axis=1)

        def step(i, carry, at=None):
            live = [at is None or 0 <= at - d < NG for d in range(DEPTH + 1)]
            def heads(d):
                return [((i - d) * G + e, ((i - d) & 1) * G + e) for e in range(G)]
            if live[0]:
                for h, sl in heads(0):
                    scores(h, sl)
            if live[3]:
                for h, sl in heads(3):
                    head_out(sl)
            if live[2]:
                for h, sl in heads(2):
                    p_times_v(h, sl)
            if live[4]:
                tot = None
                for h, sl in heads(4):
                    y = project(h, sl)
                    tot = y if tot is None else tot + y
                accb[...] = accb[...] + tot
            if live[1]:
                for h, sl in heads(1):
                    softmax(sl)
            return carry

        def wait_v(g0):
            if g0 == 0:
                @pl.when(jnp.logical_and(first, b < B - 1))
                def _():
                    wait_kv(vbuf, 1 + B + b, b, 0, H)
            for (hh, n), sem in zip(V_LAST, SEM_V_LAST):
                if hh // G == g0:
                    @pl.when(jnp.logical_and(first, b == B - 1))
                    def _():
                        wait_kv(vbuf, sem, b, hh, n)

        accb[...] = jnp.zeros((8, D), F32)
        v_starts = sorted({h0 // G for h0, _ in V_LAST})
        i = 0
        while i < NG + DEPTH:
            if i - V_STAGE in v_starts:
                wait_v(i - V_STAGE)
            nxt = min([h0 + V_STAGE for h0 in v_starts if h0 + V_STAGE > i] + [NG])
            if DEPTH <= i < NG and nxt - i >= 2:
                lax.fori_loop(i, nxt, step, 0)
                i = nxt
            else:
                step(i, 0, at=i)
                i += 1

        x = x + jnp.sum(accb[...], axis=0, keepdims=True)
        mean, rstd = _ln_stats(x)
        xn = ((x - mean) * rstd).astype(BF).astype(F32)
        r = jnp.sum(xn * wr32, axis=-1, keepdims=True)
        xt = [_with_ones(a) for a in _tiles(x)]
        NF, NO = F // 128, D // 128
        gu, hs, ys = {}, {}, {}

        def f_result(key, res):
            kind, n, k = key
            if kind < 2:
                gu[kind, n] = res if k == 0 else gu[kind, n] + res
                if k == KT - 1:
                    gu[kind, n] = (gu[kind, n][0:8] - mean * gu[kind, n][8:16]) * rstd
                    if kind == 1:
                        g, u = gu[0, n], gu[1, n]
                        hs[n] = _dup16(g * jax.nn.sigmoid(g) * u)
            else:
                ys[n] = res[0:8] if n not in ys else ys[n] + res[0:8]

        for n in range(NF):
            for kind, w in ((0, wg), (1, wu)):
                for k in range(KT):
                    f_result((kind, n, k), _dot(xt[k], w[k * 128:(k + 1) * 128, n * 128:(n + 1) * 128]))
        for k in range(NF):
            for n in range(NO):
                f_result((2, n, k), _dot(hs[k], wd[k * 128:(k + 1) * 128, n * 128:(n + 1) * 128]))
        y = jnp.concatenate([ys[n] for n in range(NO)], axis=1) * jax.nn.sigmoid(r)
        x = x + (xn + (xn * 0.0 + y))
        xs[pl.ds(b, 1), :] = x[0:1, :]
        return carry

    lax.fori_loop(0, 2 * B, layer, 0)
    out_ref[...] = xs[0:B, :].astype(BF)


@jax.jit
def pallas_interleave_layers__sliding_block_cached__moe_arch_mod__decode_kernel(
    A_x, A_k_cache, A_v_cache, A_wq, A_wo, B_x, B_w_r, B_w_gate, B_w_up, B_w_down
):
    del B_x
    kt = jnp.swapaxes(A_k_cache, 2, 3)
    vt = jnp.swapaxes(A_v_cache, 2, 3)
    anyspec = pl.BlockSpec(memory_space=pl.ANY)
    out = pl.pallas_call(
        _kernel,
        out_shape=jax.ShapeDtypeStruct((B, D), BF),
        grid=(1,),
        in_specs=[anyspec] * 9,
        out_specs=pl.BlockSpec(memory_space=pltpu.VMEM),
        scratch_shapes=[
            pltpu.VMEM((B, D), BF),
            pltpu.VMEM((B * H, NC, DH, 128), BF),
            pltpu.VMEM((B * H, NC, DH, 128), BF),
            pltpu.VMEM((D, H * DH), BF),
            pltpu.VMEM((H * DH, D), BF),
            pltpu.VMEM((D // 128, H * DH, 128), BF),
            pltpu.VMEM((D,), BF),
            pltpu.VMEM((D, F), BF),
            pltpu.VMEM((D, F), BF),
            pltpu.VMEM((F, D), BF),
            pltpu.VMEM((8, D), F32),
            pltpu.VMEM((8, D), F32),
            pltpu.VMEM((8, 128), jnp.uint32),
            pltpu.VMEM((H, 2, 8, 128), jnp.uint32),
            pltpu.VMEM((2 * G, 8, 128), F32),
            pltpu.VMEM((2 * G, 8, W), F32),
            pltpu.VMEM((2 * G, 8, 128), F32),
            pltpu.VMEM((2 * G, 8, W), F32),
            pltpu.VMEM((2 * G, 8, 128), F32),
            pltpu.VMEM((2 * G, DH, 128), F32),
            pltpu.VMEM((2 * G, 2, 8, 128), jnp.uint32),
            pltpu.SemaphoreType.DMA((NSEM,)),
        ],
        compiler_params=pltpu.CompilerParams(vmem_limit_bytes=127 * 1024 * 1024),
    )(A_x.reshape(B, D), kt, vt, A_wq, A_wo, B_w_r, B_w_gate, B_w_up, B_w_down)
    return out.reshape(B, 1, D)
```

```python
import functools

import jax
import jax.numpy as jnp
from jax import lax
import jax.experimental.pallas as pl
import jax.experimental.pallas.tpu as pltpu

B, D, H, DH, SK, W, F = 4, 640, 32, 192, 4096, 1024, 1536
NC = W // 128
SCALE = DH ** -0.5
LOG2E = 1.4426950408889634
EPS = 1e-5
BF = jnp.bfloat16
F32 = jnp.float32

V_LAST = ((0, 16), (16, 8), (24, 4), (28, 2), (30, 1), (31, 1))
V_LAST_ISSUE = 2 * (B - 2)
SEM_W = 0
SEM_K = tuple(1 + b for b in range(B))
SEM_V = tuple(1 + B + b for b in range(B - 1))
SEM_V_LAST = (SEM_V[0], SEM_V[1], SEM_K[0], SEM_K[1], SEM_W, 2 * B)
NSEM = 2 * B + 1

WO_TILES = ((0,), (1,), (2,), (3,), (4,), (0, 1), (2, 3), (4, 4))
G = 2
ORDER = (("k", 0), ("k", 1), ("w", 0), ("x", 0), ("x", 1), ("v", 0), ("w", 1), ("v", 1), ("s", 0), ("s", 1))
NG = H // G
DEPTH = 4
V_STAGE = 2


def _ln_stats(x):
    t = [x[:, i:i + 128] for i in range(0, x.shape[1], 128)]
    s1 = functools.reduce(jnp.add, t)
    s2 = functools.reduce(jnp.add, [a * a for a in t])
    n = x.shape[1]
    m = jnp.sum(s1, axis=-1, keepdims=True) * (1.0 / n)
    q = jnp.sum(s2, axis=-1, keepdims=True) * (1.0 / n)
    v = jnp.maximum(q - m * m, 0.0)
    return m, lax.rsqrt(v + EPS)


def _bf(u):
    return pltpu.bitcast(u, BF)


def _u32(x):
    return pltpu.bitcast(x.astype(BF), jnp.uint32)


def _tiles(a):
    return [a[:, i:i + 128] for i in range(0, a.shape[1], 128)]


def _dup16(a):
    return jnp.concatenate([a, a], axis=0).astype(BF)


def _with_ones(a):
    return jnp.concatenate([a, jnp.ones_like(a)], axis=0).astype(BF)


def _dot(a, b):
    return jnp.dot(a, b, preferred_element_type=F32)


def _kernel(x_hbm, k_hbm, v_hbm, wq_hbm, wo_hbm, wr_hbm, wg_hbm, wu_hbm, wd_hbm,
            out_ref,
            xb, kbuf, vbuf, wq, wo_nat, wo, wr, wg, wu, wd,
            xs, accb, onesb, qbuf, ilbuf, sbuf, mbuf, pbuf, lbuf, abuf, obuf, sems):
    weights = [pltpu.make_async_copy(s, d, sems.at[SEM_W]) for s, d in (
        (x_hbm, xb), (wr_hbm, wr), (wq_hbm, wq), (wo_hbm, wo_nat), (wg_hbm, wg), (wu_hbm, wu), (wd_hbm, wd))]

    def start_kv(hbm, buf, sem, b, h0, n):
        def tile(c, carry):
            pltpu.make_async_copy(
                hbm.at[b, pl.ds(h0, n), :, pl.ds(pl.multiple_of(SK - W + c * 128, 128), 128)],
                buf.at[pl.ds(b * H + h0, n), c], sems.at[sem]).start()
            return carry
        lax.fori_loop(0, NC, tile, 0)

    def wait_kv(buf, sem, b, h0, n):
        whole = buf.at[pl.ds(b * H + h0, n)]
        pltpu.make_async_copy(whole, whole, sems.at[sem]).wait()

    for c in weights:
        c.start()
    for b in range(B):
        start_kv(k_hbm, kbuf, SEM_K[b], b, 0, H)
        if b < B - 1:
            start_kv(v_hbm, vbuf, SEM_V[b], b, 0, H)
    for c in weights:
        c.wait()

    xs[...] = jnp.zeros((8, D), F32)
    xs[0:B, :] = xb[...].astype(F32)
    wr32 = jnp.broadcast_to(wr[...].astype(F32).reshape(1, D), (8, D))
    onesb[...] = pltpu.bitcast(jnp.ones((16, 128), BF), jnp.uint32)

    def retile(i, carry):
        r0 = pl.multiple_of(i * 256, 256)
        for n in range(D // 128):
            wo[n, pl.ds(r0, 256), :] = wo_nat[pl.ds(r0, 256), n * 128:(n + 1) * 128]
        return carry
    lax.fori_loop(0, H * DH // 256, retile, 0)

    k32 = kbuf.bitcast(jnp.uint32)
    v32 = vbuf.bitcast(jnp.uint32)
    wo32 = wo.bitcast(jnp.uint32)

    def layer(it, carry):
        b = it // 2
        first = (it % 2) == 0

        @pl.when(it == V_LAST_ISSUE)
        def _():
            for (h0, n), sem in zip(V_LAST, SEM_V_LAST):
                start_kv(v_hbm, vbuf, sem, B - 1, h0, n)

        @pl.when(first)
        def _():
            wait_kv(kbuf, 1 + b, b, 0, H)

        x = jnp.broadcast_to(xs[pl.ds(b, 1), :], (8, D))
        lo_half = lax.broadcasted_iota(jnp.int32, (8, 128), 1) < 64
        KT = D // 128

        mean, rstd = _ln_stats(x)
        xt = [_with_ones(a) for a in _tiles(x)]
        part, done = {}, set()

        def q_pair(j, t0, t1, t2):
            r1 = pltpu.roll(t1, 64, 1)
            r2 = pltpu.roll(t2, 64, 1)
            qbuf[2 * j, 0] = _u32(_dup16(t0))
            qbuf[2 * j, 1] = _u32(jnp.concatenate([jnp.where(lo_half, t1, 0.0), jnp.where(lo_half, 0.0, r1)], axis=0))
            qbuf[2 * j + 1, 0] = _u32(_dup16(jnp.where(lo_half, r1, r2)))
            qbuf[2 * j + 1, 1] = _u32(jnp.concatenate([jnp.where(lo_half, r2, 0.0), jnp.where(lo_half, 0.0, t2)], axis=0))

        def q_result(key, res):
            n, k = key
            part[n] = res if k == 0 else part[n] + res
            if k == KT - 1:
                part[n] = (part[n][0:8] - mean * part[n][8:16]) * (rstd * (SCALE * LOG2E))
                done.add(n)
                j = n // 3
                if all(3 * j + t in done for t in range(3)):
                    q_pair(j, part[3 * j], part[3 * j + 1], part[3 * j + 2])

        for n in range(H * DH // 128):
            for k in range(KT):
                q_result((n, k), _dot(xt[k], wq[k * 128:(k + 1) * 128, n * 128:(n + 1) * 128]))

        def k_rhs(h, m, j):
            if j < 2:
                return _bf(k32[b * H + h, 2 * m + j, 0:64, :])
            return jnp.concatenate([_bf(k32[b * H + h, 2 * m, 64:96, :]), _bf(k32[b * H + h, 2 * m + 1, 64:96, :])], axis=0)

        def wo_rhs(h, j):
            r0 = h * (DH // 2)
            if not isinstance(h, int):
                r0 = pl.multiple_of(r0, 32)
            t = WO_TILES[j]
            if len(t) == 1:
                return _bf(wo32[t[0], pl.ds(r0, 64), :])
            return jnp.concatenate([_bf(wo32[t[0], pl.ds(r0 + 64, 32), :]), _bf(wo32[t[1], pl.ds(r0 + 64, 32), :])], axis=0)

        def scores(h, sl):
            ql = [_bf(qbuf[h, 0]), _bf(qbuf[h, 1])]
            mx = None
            for m in range(NC // 2):
                hf = _dot(ql[1], k_rhs(h, m, 2))
                for j in range(2):
                    sc = _dot(ql[0], k_rhs(h, m, j))[0:8] + hf[8 * j:8 * j + 8]
                    c = 2 * m + j
                    sbuf[sl, :, c * 128:(c + 1) * 128] = sc
                    mx = sc if mx is None else jnp.maximum(mx, sc)
            mbuf[sl] = mx

        def softmax(sl):
            mx = jnp.max(mbuf[sl], axis=-1, keepdims=True)
            ps = None
            for c in range(NC):
                p = jnp.exp2(sbuf[sl, :, c * 128:(c + 1) * 128] - mx)
                pbuf[sl, :, c * 128:(c + 1) * 128] = p
                ps = p if ps is None else ps + p
            lbuf[sl] = ps

        def p_times_v(h, sl):
            p = pbuf[sl]
            l = jnp.sum(lbuf[sl], axis=-1, keepdims=True)
            ilbuf[sl] = jnp.broadcast_to(1.0 / l, (8, 128))
            for r in range(DH // 16):
                a = None
                for c in range(NC):
                    t = vbuf[b * H + h, c, 16 * r:16 * r + 16, :].astype(F32).reshape(2, 8, 128) * p[None, :, c * 128:(c + 1) * 128]
                    a = t if a is None else a + t
                abuf[sl, 16 * r:16 * r + 16, :] = a.reshape(16, 128)

        lane = lax.broadcasted_iota(jnp.int32, (8, 128), 1)
        grp = lane // 8
        diag = lax.broadcasted_iota(jnp.int32, (8, 128), 0) == lane % 8

        def head_out(sl):
            d0 = d1 = jnp.zeros((8, 128), F32)
            for g in range(DH // 8):
                red = jnp.sum(abuf[sl, 8 * g:8 * g + 8, :], axis=-1, keepdims=True)
                if g < 16:
                    d0 = jnp.where(grp == g, red, d0)
                else:
                    d1 = jnp.where(grp % 8 == g - 16, red, d1)
            il = ilbuf[sl]
            o1 = d1 * il
            obuf[sl, 0] = _u32(_dup16(jnp.where(diag, d0 * il, 0.0)))
            obuf[sl, 1] = _u32(jnp.concatenate([jnp.where(diag & lo_half, o1, 0.0), jnp.where(diag & ~lo_half, o1, 0.0)], axis=0))

        def project(h, sl):
            ol = [_bf(obuf[sl, 0]), _bf(obuf[sl, 1])]
            outs = [None] * (D // 128)
            for j, t in enumerate(WO_TILES):
                r = _dot(ol[len(t) - 1], wo_rhs(h, j))
                pieces = [(t[0], r[0:8])] if (len(t) == 1 or t[0] == t[1]) else [(t[0], r[0:8]), (t[1], r[8:16])]
                for n, v in pieces:
                    outs[n] = v if outs[n] is None else outs[n] + v
            return jnp.concatenate(outs, axis=1)

        def step(i, carry, at=None):
            live = [at is None or 0 <= at - d < NG for d in range(DEPTH + 1)]
            def heads(d):
                return [((i - d) * G + e, ((i - d) & 1) * G + e) for e in range(G)]
            tot = None
            for what, e in ORDER:
                d = {"k": 0, "s": 1, "v": 2, "x": 3, "w": 4}[what]
                if not live[d]:
                    continue
                h, sl = heads(d)[e]
                if what == "k":
                    scores(h, sl)
                elif what == "s":
                    softmax(sl)
                elif what == "v":
                    p_times_v(h, sl)
                elif what == "x":
                    head_out(sl)
                else:
                    y = project(h, sl)
                    tot = y if tot is None else tot + y
            if tot is not None:
                accb[...] = accb[...] + tot
            return carry

        def wait_v(g0):
            if g0 == 0:
                @pl.when(jnp.logical_and(first, b < B - 1))
                def _():
                    wait_kv(vbuf, 1 + B + b, b, 0, H)
            for (hh, n), sem in zip(V_LAST, SEM_V_LAST):
                if hh // G == g0:
                    @pl.when(jnp.logical_and(first, b == B - 1))
                    def _():
                        wait_kv(vbuf, sem, b, hh, n)

        accb[...] = jnp.zeros((8, D), F32)
        v_starts = sorted({h0 // G for h0, _ in V_LAST})
        i = 0
        while i < NG + DEPTH:
            if i - V_STAGE in v_starts:
                wait_v(i - V_STAGE)
            nxt = min([h0 + V_STAGE for h0 in v_starts if h0 + V_STAGE > i] + [NG])
            if DEPTH <= i < NG and nxt - i >= 2:
                lax.fori_loop(i, nxt, step, 0)
                i = nxt
            else:
                step(i, 0, at=i)
                i += 1

        x = x + jnp.sum(accb[...], axis=0, keepdims=True)
        mean, rstd = _ln_stats(x)
        xn = ((x - mean) * rstd).astype(BF).astype(F32)
        r = jnp.sum(xn * wr32, axis=-1, keepdims=True)
        xt = [_with_ones(a) for a in _tiles(x)]
        NF, NO = F // 128, D // 128
        gu, hs, ys = {}, {}, {}

        def f_result(key, res):
            kind, n, k = key
            if kind < 2:
                gu[kind, n] = res if k == 0 else gu[kind, n] + res
                if k == KT - 1:
                    gu[kind, n] = (gu[kind, n][0:8] - mean * gu[kind, n][8:16]) * rstd
                    if kind == 1:
                        g, u = gu[0, n], gu[1, n]
                        hs[n] = _dup16(g * jax.nn.sigmoid(g) * u)
            else:
                ys[n] = res[0:8] if n not in ys else ys[n] + res[0:8]

        for n in range(NF):
            for kind, w in ((0, wg), (1, wu)):
                for k in range(KT):
                    f_result((kind, n, k), _dot(xt[k], w[k * 128:(k + 1) * 128, n * 128:(n + 1) * 128]))
        for k in range(NF):
            for n in range(NO):
                f_result((2, n, k), _dot(hs[k], wd[k * 128:(k + 1) * 128, n * 128:(n + 1) * 128]))
        y = jnp.concatenate([ys[n] for n in range(NO)], axis=1) * jax.nn.sigmoid(r)
        x = x + (xn + (xn * 0.0 + y))
        xs[pl.ds(b, 1), :] = x[0:1, :]
        return carry

    lax.fori_loop(0, 2 * B, layer, 0)
    out_ref[...] = xs[0:B, :].astype(BF)


@jax.jit
def pallas_interleave_layers__sliding_block_cached__moe_arch_mod__decode_kernel(
    A_x, A_k_cache, A_v_cache, A_wq, A_wo, B_x, B_w_r, B_w_gate, B_w_up, B_w_down
):
    del B_x
    kt = jnp.swapaxes(A_k_cache, 2, 3)
    vt = jnp.swapaxes(A_v_cache, 2, 3)
    anyspec = pl.BlockSpec(memory_space=pl.ANY)
    out = pl.pallas_call(
        _kernel,
        out_shape=jax.ShapeDtypeStruct((B, D), BF),
        grid=(1,),
        in_specs=[anyspec] * 9,
        out_specs=pl.BlockSpec(memory_space=pltpu.VMEM),
        scratch_shapes=[
            pltpu.VMEM((B, D), BF),
            pltpu.VMEM((B * H, NC, DH, 128), BF),
            pltpu.VMEM((B * H, NC, DH, 128), BF),
            pltpu.VMEM((D, H * DH), BF),
            pltpu.VMEM((H * DH, D), BF),
            pltpu.VMEM((D // 128, H * DH, 128), BF),
            pltpu.VMEM((D,), BF),
            pltpu.VMEM((D, F), BF),
            pltpu.VMEM((D, F), BF),
            pltpu.VMEM((F, D), BF),
            pltpu.VMEM((8, D), F32),
            pltpu.VMEM((8, D), F32),
            pltpu.VMEM((8, 128), jnp.uint32),
            pltpu.VMEM((H, 2, 8, 128), jnp.uint32),
            pltpu.VMEM((2 * G, 8, 128), F32),
            pltpu.VMEM((2 * G, 8, W), F32),
            pltpu.VMEM((2 * G, 8, 128), F32),
            pltpu.VMEM((2 * G, 8, W), F32),
            pltpu.VMEM((2 * G, 8, 128), F32),
            pltpu.VMEM((2 * G, DH, 128), F32),
            pltpu.VMEM((2 * G, 2, 8, 128), jnp.uint32),
            pltpu.SemaphoreType.DMA((NSEM,)),
        ],
        compiler_params=pltpu.CompilerParams(vmem_limit_bytes=127 * 1024 * 1024),
    )(A_x.reshape(B, D), kt, vt, A_wq, A_wo, B_w_r, B_w_gate, B_w_up, B_w_down)
    return out.reshape(B, 1, D)
```
